```python
import os as _os
_os.environ.setdefault('JAX_PLATFORMS', 'cpu')
import jax
import jax.numpy as jnp

def _softmax(x, axis=-1):
    return jax.nn.softmax(x, axis=axis)

def _gelu(x):
    return jax.nn.gelu(x, approximate=True)

def _silu(x):
    return jax.nn.silu(x)

def _sigmoid(x):
    return jax.nn.sigmoid(x)

def _layernorm(x, axis=-1, eps=1e-05):
    m = jnp.mean(x, axis=axis, keepdims=True)
    v = jnp.var(x, axis=axis, keepdims=True)
    return (x - m) / jnp.sqrt(v + eps)

def _scatter_add(tgt, idx, src, axis=0):
    return tgt.at[idx].add(src)

def _segment_sum(src, seg, n):
    return jax.ops.segment_sum(src, seg, n)

class _Rng:

    def __init__(self, key):
        self._k = key

    def _next(self):
        self._k, sub = jax.random.split(self._k)
        return sub

    def normal(self, shape):
        return jax.random.normal(self._next(), shape, dtype=jnp.bfloat16)

    def randint(self, lo, hi, shape):
        return jax.random.randint(self._next(), shape, lo, hi, dtype=jnp.int32)

    def uniform(self, shape, lo=0.0, hi=1.0):
        return jax.random.uniform(self._next(), shape, jnp.bfloat16, lo, hi)

    def permutation(self, n):
        return jax.random.permutation(self._next(), n)
kernel_name = 'recurrent_scan__memory_aug_recurrent_mem_tr__mixer_gmlp__prompt'

def setup_inputs():
    _rng = _Rng(jax.random.key(int.from_bytes(__import__("os").urandom(4), "little")))
    _w = lambda a: (lambda t: t.astype(jnp.bfloat16) if jnp.issubdtype(t.dtype, jnp.floating) else t)(jnp.asarray(a))

    def _A_setup():
        B, S, Dm = (1, 2048, 640)
        H, Dh = (32, 128)
        M, seg = (8, 32)
        seg = min(seg, S)
        S = S // seg * seg
        return {'x': _w((lambda *s: _rng.normal(s) * 0.05)(B, S, Dm)), 'mem0': _w((lambda *s: _rng.normal(s) * 0.1)(B, M, Dm)), 'Wq': _w((lambda *s: _rng.normal(s) * 1.6)(Dm, H, Dh) * Dm ** (-0.5)), 'Wk': _w((lambda *s: _rng.normal(s) * 1.6)(Dm, H, Dh) * Dm ** (-0.5)), 'Wv': _w((lambda *s: _rng.normal(s) * 0.1)(Dm, H, Dh) * Dm ** (-0.5)), 'Wo': _w((lambda *s: _rng.normal(s) * 0.1)(H, Dh, Dm) * (H * Dh) ** (-0.5)), 'seg_len': seg}
    _A_in = _A_setup()

    def _B_setup():
        B, S, D, F = (1, 2048, 640, 1728)
        Fh = F // 2
        return {'x': _w((lambda *s: _rng.normal(s) * 0.05)(B, S, D)), 'w_in': _w((lambda *s: _rng.normal(s) * 0.8)(D, 2 * Fh)), 'w_sp': _w(0.01 * (lambda *s: _rng.normal(s) * 0.8)(S, S)), 'b_sp': _w(1.0 + 0.01 * (lambda *s: _rng.normal(s) * 0.05)(S)), 'w_out': _w((lambda *s: _rng.normal(s) * 0.05)(Fh, D))}
    _B_in = _B_setup()
    return {'A_x': _A_in['x'], 'A_mem0': _A_in['mem0'], 'A_Wq': _A_in['Wq'], 'A_Wk': _A_in['Wk'], 'A_Wv': _A_in['Wv'], 'A_Wo': _A_in['Wo'], 'A_seg_len': _A_in['seg_len'], 'B_x': _B_in['x'], 'B_w_in': _B_in['w_in'], 'B_w_sp': _B_in['w_sp'], 'B_b_sp': _B_in['b_sp'], 'B_w_out': _B_in['w_out']}

def reference(A_x, A_mem0, A_Wq, A_Wk, A_Wv, A_Wo, A_seg_len, B_x, B_w_in, B_w_sp, B_b_sp, B_w_out):

    def _A_ref(x, mem0, Wq, Wk, Wv, Wo, seg_len):
        B, S, Dm = x.shape
        H, Dh = (Wq.shape[1], Wq.shape[2])
        M = mem0.shape[1]
        scale = Dh ** (-0.5)
        n_seg = S // seg_len
        L = M + seg_len
        idx = jnp.arange(L)
        mask = (idx[:, None] < M) | (idx[:, None] >= idx[None, :])
        mem = mem0
        outs = []
        for s in range(n_seg):
            xs = x[:, s * seg_len:(s + 1) * seg_len, :].copy()
            h = jnp.concatenate([mem, xs], axis=1)
            q = jnp.einsum('btd,dhe->bhte', h, Wq)
            k = jnp.einsum('btd,dhe->bhte', h, Wk)
            v = jnp.einsum('btd,dhe->bhte', h, Wv)
            scores = jnp.einsum('bhqe,bhke->bhqk', q, k) * scale
            scores = jnp.where(mask[None, None], scores, -1000000000.0)
            p = _softmax(scores, axis=-1)
            o = jnp.einsum('bhqk,bhke->bhqe', p, v)
            o = jnp.einsum('bhte,hed->btd', o, Wo)
            mem = o[:, :M, :].copy()
            outs.append(o[:, M:, :])
        return jnp.concatenate(outs, axis=1)

    def _B_ref(x, w_in, w_sp, b_sp, w_out):
        B, S, D = x.shape
        F = w_in.shape[-1]
        Fh = F // 2
        z = _gelu(jnp.einsum('bsd,df->bsf', x, w_in))
        z1 = z[..., :Fh].copy()
        z2 = _layernorm(z[..., Fh:], axis=-1)
        g = jnp.einsum('ts,bsf->btf', w_sp, z2) + b_sp[None, :, None]
        return jnp.einsum('bsf,fd->bsd', z1 * g, w_out)
    x = A_x
    xn = _layernorm(x, axis=-1)
    s = _A_ref(xn, A_mem0, A_Wq, A_Wk, A_Wv, A_Wo, A_seg_len)
    g = _silu(_B_ref(xn, B_w_in, B_w_sp, B_b_sp, B_w_out))
    return x + s * g
```

```python
import functools
import math
import jax
import jax.numpy as jnp
from jax import lax
import jax.experimental.pallas as pl
import jax.experimental.pallas.tpu as pltpu

F32 = jnp.float32
BF16 = jnp.bfloat16
U32 = jnp.uint32
NT = (((1,), (1,)), ((), ()))


def _ln(x, n):
    m = jnp.sum(x, axis=-1, keepdims=True) * (1.0 / n)
    d = x - m
    v = jnp.sum(d * d, axis=-1, keepdims=True) * (1.0 / n)
    return d * lax.rsqrt(v + 1e-5)


def _gelu(x):
    c = math.sqrt(2.0 / math.pi)
    return 0.5 * x * (1.0 + jnp.tanh(c * (x + 0.044715 * (x * x * x))))


def _dot(a, b):
    return jnp.dot(a, b, preferred_element_type=F32)


def _bf(u32_val):
    return pltpu.bitcast(u32_val, BF16)


@functools.partial(jax.jit, static_argnames=("A_seg_len",))
def pallas_recurrent_scan__memory_aug_recurrent_mem_tr__mixer_gmlp__prompt_kernel(A_x, A_mem0, A_Wq, A_Wk, A_Wv, A_Wo, A_seg_len, B_x, B_w_in, B_w_sp, B_b_sp, B_w_out):
    del B_x
    _, S, D = A_x.shape
    H, Dh = A_Wq.shape[1], A_Wq.shape[2]
    M = A_mem0.shape[1]
    SEG = int(A_seg_len)
    NSEG = S // SEG
    L = SEG + M
    F = B_w_in.shape[1]
    Fh = F // 2
    scale = Dh ** -0.5
    NP = H // 2
    CH = 256
    PADR = H + 8
    D2 = D // 2

    x2 = A_x.reshape(S, D)
    mem0 = A_mem0.reshape(M, D)
    wq = A_Wq.reshape(D2, 2 * H, Dh)
    wk = A_Wk.reshape(D2, 2 * H, Dh)
    wv = A_Wv.reshape(D2, 2 * H, Dh)
    wo = A_Wo.reshape(H * Dh, D)
    winT = B_w_in.T
    b2 = B_b_sp.reshape(S // 128, 128)

    def kern(x_hbm, mem0_ref, wq_hbm, wk_hbm, wv_hbm, wo_hbm, winT_hbm, wsp_hbm, b_ref, wout_hbm,
             o_hbm,
             x_ref, winT_ref, raw_ref, wo_ref, wout_ref, wsp_ref, o_ref,
             xn_ref, z1_ref, z2_ref, wqkv_ref, bcol_ref, mem_ref, sem, osem):
        raw3 = raw_ref.reshape(3 * D2, PADR, Dh)
        cp_x = pltpu.make_async_copy(x_hbm, x_ref, sem.at[0])
        cp_win = pltpu.make_async_copy(winT_hbm.bitcast(U32), winT_ref, sem.at[1])
        cp_w = [pltpu.make_async_copy(w.bitcast(U32), raw3.at[j * D2:(j + 1) * D2, 0:H, :], sem.at[2 + j])
                for j, w in enumerate((wq_hbm, wk_hbm, wv_hbm))]
        cp_wo = pltpu.make_async_copy(wo_hbm.bitcast(U32), wo_ref, sem.at[5])
        cp_wout = pltpu.make_async_copy(wout_hbm.bitcast(U32), wout_ref, sem.at[6])
        cp_wsp = pltpu.make_async_copy(wsp_hbm.bitcast(U32), wsp_ref, sem.at[7])
        cp_x.start()
        cp_win.start()
        for c in cp_w:
            c.start()
        cp_wo.start()
        cp_wout.start()
        cp_wsp.start()

        bT = jnp.concatenate([b_ref[...].astype(F32), jnp.zeros((128 - S // 128, 128), F32)], axis=0).T
        for i in range(S // 128):
            bcol_ref[i * 128:(i + 1) * 128, :] = jnp.broadcast_to(bT[:, i:i + 1], (128, 128))
        mem_ref[...] = mem0_ref[...].astype(F32)

        cp_x.wait()
        cp_win.wait()

        def pro(c, carry):
            r = pl.ds(pl.multiple_of(c * CH, CH), CH)
            r2 = pl.ds(pl.multiple_of(c * (CH // 2), CH // 2), CH // 2)
            xnf = _ln(x_ref[r, :].astype(F32), D)
            xn = xnf.astype(BF16)
            xn_ref[r, :] = xn.astype(F32)
            za = _gelu(lax.dot_general(xn, _bf(winT_ref[:Fh // 2, :]), NT, preferred_element_type=F32))
            z1_ref[r2, :] = pltpu.bitcast(za.astype(BF16), U32)
            zb = _gelu(lax.dot_general(xn, _bf(winT_ref[Fh // 2:, :]), NT, preferred_element_type=F32))
            z2_ref[r2, :] = pltpu.bitcast(_ln(zb, Fh).astype(BF16), U32)
            return carry
        lax.fori_loop(0, S // CH, pro, 0)

        DC = 32
        for j in range(3):
            cp_w[j].wait()
            def rl(c, carry, j=j):
                sub = raw_ref.at[pl.ds(pl.multiple_of((j * D2 + c * DC) * PADR, 8), DC * PADR), :]
                rows = pl.ds(pl.multiple_of(c * DC, DC), DC)
                for p in range(NP):
                    a = sub[pl.ds(p, DC, stride=PADR), :]
                    b = sub[pl.ds(NP + p, DC, stride=PADR), :]
                    lo = (a & U32(0xFFFF)) | (b << 16)
                    hi = (a >> 16) | (b & U32(0xFFFF0000))
                    wqkv_ref[p, rows, (2 * j) * Dh:(2 * j + 1) * Dh] = lo
                    wqkv_ref[p, rows, (2 * j + 1) * Dh:(2 * j + 2) * Dh] = hi
                return carry
            lax.fori_loop(0, D2 // DC, rl, 0)
        cp_wo.wait()
        cp_wout.wait()
        cp_wsp.wait()

        ri = lax.broadcasted_iota(jnp.int32, (2 * L, 2 * L), 0)
        ci = lax.broadcasted_iota(jnp.int32, (2 * L, 2 * L), 1)
        rh = ri >= L
        chd = ci >= L
        rr = jnp.where(rh, ri - L, ri)
        cc = jnp.where(chd, ci - L, ci)
        same = rh == chd
        valid = same & ((rr >= SEG) | (cc >= SEG) | (rr >= cc))
        fill = jnp.where(same, -1e9, -jnp.inf).astype(F32)

        def attn_fns(qkv, pm, oc):
            def score(p):
                q2, k2, _ = qkv[p]
                sc = lax.dot_general(q2, k2, NT, preferred_element_type=F32) * scale
                sc = jnp.where(valid, sc, fill)
                mx = jnp.max(sc, axis=-1, keepdims=True)
                e = jnp.exp(sc - mx)
                den = jnp.sum(e, axis=-1, keepdims=True)
                pm[p] = (e.astype(BF16), 1.0 / den)

            def pv(p):
                e, inv = pm[p]
                o2 = _dot(e, qkv[p][2]) * inv
                oc[p] = jnp.concatenate([o2[:L], o2[L:]], axis=1)
            return score, pv

        def heads(t):
            return tuple(
                jnp.concatenate([t[:, (2 * j) * Dh:(2 * j + 1) * Dh], t[:, (2 * j + 1) * Dh:(2 * j + 2) * Dh]],
                                axis=0).astype(BF16) for j in range(3))

        def wo_dot(lhs_fn, ps, acc):
            lhs = jnp.concatenate([lhs_fn(p) for p in ps], axis=1).astype(BF16)
            t = _dot(lhs, _bf(wo_ref[ps[0] * Dh:(ps[-1] + 1) * Dh, :]))
            return t if acc is None else t + acc

        def step(it, carry):
            r0 = pl.multiple_of(it * (2 * SEG), 2 * SEG)
            r = pl.ds(r0, 2 * SEG)
            rh2 = pl.ds(pl.multiple_of(it * SEG, SEG), SEG)
            ha = jnp.concatenate([xn_ref[pl.ds(r0, SEG + M), :], mem_ref[...]], axis=0).astype(BF16)
            qkv, pm, oca, saved = {}, {}, {}, {}
            score, pv = attn_fns(qkv, pm, oca)

            def proj_a(p):
                t = _dot(ha, _bf(wqkv_ref[p]))
                saved[p] = t[SEG:SEG + M]
                qkv[p] = heads(jnp.concatenate([t[:SEG], t[SEG + M:]], axis=0))

            for i in range(NP):
                proj_a(i)
                if i >= 1:
                    score(i - 1)
                if i >= 3:
                    pv(i - 3)
            lhs_a = lambda p: jnp.concatenate([oca[p][:SEG - M], oca[p][SEG:]], axis=0)
            acc = wo_dot(lhs_a, [0, 1, 2], None)
            score(NP - 1)
            pv(NP - 3)
            acc = wo_dot(lhs_a, [3, 4, 5], acc)
            pv(NP - 2)
            acc = wo_dot(lhs_a, [6, 7, 8, 9], acc)
            pv(NP - 1)
            acc = wo_dot(lhs_a, [10, 11, 12, 13, 14], acc)
            acc_a = wo_dot(lhs_a, [15], acc)
            mem_b = acc_a[SEG - M:].astype(BF16).astype(F32)
            g = _dot(_bf(wsp_ref[rh2, :]), _bf(z2_ref[...])) + bcol_ref[r, 0:1]
            u = (_bf(z1_ref[rh2, :]).astype(F32) * g).astype(BF16)
            hb = jnp.concatenate([xn_ref[pl.ds(r0 + SEG + M, SEG - M), :], mem_b], axis=0).astype(BF16)
            qkv, pm, ocb = {}, {}, {}
            score, pv = attn_fns(qkv, pm, ocb)

            def proj_b(p):
                t = _dot(hb, _bf(wqkv_ref[p]))
                qkv[p] = heads(jnp.concatenate([saved[p], t], axis=0))

            for i in range(NP):
                proj_b(i)
                if i >= 1:
                    score(i - 1)
                if i >= 3:
                    pv(i - 3)
            lhs_b = lambda p: jnp.concatenate([oca[p][SEG - M:SEG], ocb[p]], axis=0)
            y = _dot(u, _bf(wout_ref[...]))
            score(NP - 1)
            pv(NP - 3)
            acc = wo_dot(lhs_b, [0, 1, 2], None)
            pv(NP - 2)
            acc = wo_dot(lhs_b, [3, 4, 5, 6], acc)
            pv(NP - 1)
            acc = wo_dot(lhs_b, [7, 8, 9, 10, 11, 12, 13, 14], acc)
            acc_b = wo_dot(lhs_b, [15], acc)
            mem_ref[...] = acc_b[SEG + M:].astype(BF16).astype(F32)
            sa = jnp.concatenate([acc_a[:SEG - M], acc_b[:SEG + M]], axis=0)
            gate = y * (1.0 / (1.0 + jnp.exp(-y)))
            o_ref[r, :] = (x_ref[r, :].astype(F32) + sa * gate).astype(BF16)
            pltpu.make_async_copy(o_ref.at[r, :], o_hbm.at[r, :], osem).start()
            return carry
        lax.fori_loop(0, NSEG // 2, step, 0)
        pltpu.make_async_copy(o_ref, o_hbm, osem).wait()

    any_spec = pl.BlockSpec(memory_space=pl.ANY)
    vm_spec = pl.BlockSpec(memory_space=pltpu.VMEM)
    out = pl.pallas_call(
        kern,
        out_shape=jax.ShapeDtypeStruct((S, D), BF16),
        in_specs=[any_spec, vm_spec, any_spec, any_spec, any_spec, any_spec, any_spec, any_spec, vm_spec, any_spec],
        out_specs=any_spec,
        scratch_shapes=[
            pltpu.VMEM((S, D), BF16),
            pltpu.VMEM((F // 2, D), U32),
            pltpu.VMEM((3 * D2 * PADR, Dh), U32),
            pltpu.VMEM((H * Dh // 2, D), U32),
            pltpu.VMEM((Fh // 2, D), U32),
            pltpu.VMEM((S // 2, S), U32),
            pltpu.VMEM((S, D), BF16),
            pltpu.VMEM((S, D), F32),
            pltpu.VMEM((S // 2, Fh), U32),
            pltpu.VMEM((S // 2, Fh), U32),
            pltpu.VMEM((NP, D2, 6 * Dh), U32),
            pltpu.VMEM((S, 128), F32),
            pltpu.VMEM((M, D), F32),
            pltpu.SemaphoreType.DMA((8,)),
            pltpu.SemaphoreType.DMA,
        ],
        compiler_params=pltpu.CompilerParams(vmem_limit_bytes=110 * 1024 * 1024),
    )(x2, mem0, wq, wk, wv, wo, winT, B_w_sp, b2, B_w_out)
    return out.reshape(1, S, D)
```

```python
import functools
import math

import jax
import jax.numpy as jnp
from jax import lax
import jax.experimental.pallas as pl
import jax.experimental.pallas.tpu as pltpu

F32 = jnp.float32
BF16 = jnp.bfloat16
U32 = jnp.uint32
NT = (((1,), (1,)), ((), ()))


def _ln(x, n):
    m = jnp.sum(x, axis=-1, keepdims=True) * (1.0 / n)
    d = x - m
    v = jnp.sum(d * d, axis=-1, keepdims=True) * (1.0 / n)
    return d * lax.rsqrt(v + 1e-5)


def _gelu(x):
    c = math.sqrt(2.0 / math.pi)
    h = 0.5 * x
    return h + h * jnp.tanh(x * (c + (c * 0.044715) * (x * x)))


def _dot(a, b):
    return jnp.dot(a, b, preferred_element_type=F32)


def _dot_nt(a, b):
    return lax.dot_general(a, b, NT, preferred_element_type=F32)


def _bf(u32_val):
    return pltpu.bitcast(u32_val, BF16)


def _u32(bf_val):
    return pltpu.bitcast(bf_val, U32)


def _token(t):
    b = pltpu.bitcast(t[0:8, 0:128], U32)
    return (b >> 16) >> 16


def _after(x, tok):
    if tok is None:
        return x
    r, c = x.shape
    z = jnp.concatenate([tok] * (r // 8), axis=0)
    z = jnp.concatenate([z] * (-(-c // 128)), axis=1)[:, :c]
    return pltpu.bitcast(pltpu.bitcast(x, U32) | z, x.dtype)


def _rows(start, size, align):
    return pl.ds(pl.multiple_of(start, align), size)


@functools.partial(jax.jit, static_argnames=("SEG",))
def _run(A_x, A_mem0, A_Wq, A_Wk, A_Wv, A_Wo, B_w_in, B_w_sp, B_b_sp, B_w_out, *, SEG):
    _, S, D = A_x.shape
    H, Dh = A_Wq.shape[1], A_Wq.shape[2]
    M = A_mem0.shape[1]
    F = B_w_in.shape[1]
    assert (S, D, H, Dh, M, SEG, F) == (2048, 640, 32, 128, 8, 32, 1728) and A_x.shape[0] == 1
    NIT = S // SEG // 2
    L = SEG + M
    Fh = F // 2
    scale = Dh ** -0.5
    NP = H // 2
    D2 = D // 2
    NT7 = -(-Fh // 128)
    HC = 128
    FS = 5
    FI = (S // HC - 1) // FS
    CH = 1024
    NCH = S // CH
    UP = 512
    UC = 256
    NU = UP // UC
    BR = (S - UP) // NIT
    UNR = 2
    WS0 = UP + UNR * BR
    PG = NP // NU
    NW0 = 10

    x2 = A_x.reshape(S, D)
    mem0 = A_mem0.reshape(M, D)
    wq = A_Wq.reshape(D2, 2 * H, Dh)
    wk = A_Wk.reshape(D2, 2 * H, Dh)
    wv = A_Wv.reshape(D2, 2 * H, Dh)
    wo = A_Wo.reshape(H * Dh, D)
    winT = B_w_in.T
    b2 = B_b_sp.reshape(S // 128, 128)

    def kern(x_hbm, mem0_hbm, wq_hbm, wk_hbm, wv_hbm, wo_hbm, winT_hbm, wsp_hbm, b_hbm, wout_hbm,
             o_hbm,
             x_ref, winT_ref, w_ref, wo_ref, wout_ref, wsp_ref, o_ref,
             xn_ref, z1_ref, z2_ref, bcol_ref, mem_ref, gate_ref, tmp_ref, nxt_ref, lst_ref, xst_ref,
             mem0_ref, b_ref, xsem, wsem, sem, osem):
        w_hbm = [w.bitcast(U32) for w in (wq_hbm, wk_hbm, wv_hbm)]
        wsp32 = wsp_hbm.bitcast(U32)
        winT32 = winT_hbm.bitcast(U32)

        XB = [0, 2 * HC] + [min(2 * HC + (c + 1) * FS * HC, S) for c in range(FI)]

        def cp_x(c):
            return pltpu.make_async_copy(x_hbm.at[XB[c]:XB[c + 1], :], x_ref.at[XB[c]:XB[c + 1], :], xsem.at[c])

        def start_w(p):
            for j in range(3):
                for par in range(2):
                    pltpu.make_async_copy(w_hbm[j].at[:, par * NP + p, :],
                                          w_ref.at[6 * p + 2 * j + par], wsem.at[p // PG]).start()

        def wait_w(k):
            grp = w_ref.at[pl.ds(k * (6 * PG), 6 * PG)]
            pltpu.make_async_copy(grp, grp, wsem.at[k]).wait()

        cp_w2 = pltpu.make_async_copy(winT32.at[Fh // 2:], winT_ref.at[Fh // 2:], sem.at[0])
        cp_w1 = pltpu.make_async_copy(winT32.at[:Fh // 2], winT_ref.at[:Fh // 2], sem.at[1])
        cp_wo = pltpu.make_async_copy(wo_hbm.bitcast(U32), wo_ref, sem.at[2])
        cp_wout = pltpu.make_async_copy(wout_hbm.bitcast(U32), wout_ref, sem.at[3])
        cp_ws0 = pltpu.make_async_copy(wsp32.at[0:WS0 // 2], wsp_ref.at[0:WS0 // 2], sem.at[4])
        cp_ws1 = pltpu.make_async_copy(wsp32.at[WS0 // 2:], wsp_ref.at[WS0 // 2:], sem.at[5])
        cp_m = pltpu.make_async_copy(mem0_hbm, mem0_ref, sem.at[6])
        cp_b = pltpu.make_async_copy(b_hbm, b_ref, sem.at[7])
        cp_x(0).start()
        cp_b.start()
        cp_m.start()
        cp_w2.start()
        for c in range(1, FI + 1):
            cp_x(c).start()
        cp_w1.start()
        for p in range(NW0):
            start_w(p)
        cp_wout.start()
        cp_ws0.start()

        def loop(n, fn):
            def body(c, carry):
                fn(c)
                return carry
            lax.fori_loop(0, n, body, 0)

        def norm_slab(hrow, tok=None):
            xn = _ln(_after(x_ref[_rows(hrow * 2, 16, 16), :].astype(F32), tok), D).astype(BF16)
            xn_ref[_rows(hrow, 8, 8), :] = _u32(xn)
            return xn

        def z2_tile(xn, r, n):
            n0, n1 = n * 128, min((n + 1) * 128, Fh)
            t = _dot_nt(xn, _bf(winT_ref[(Fh + n0) // 2:(Fh + n1) // 2, :]))
            tmp_ref[r, n0:n1] = _gelu(t)
            return t

        def front2(c):
            for k in range(FI):
                @pl.when(c == k)
                def _():
                    cp_x(k + 1).wait()
            base = HC + c * (FS * HC)
            xn = _bf(nxt_ref[...])
            REL = [-3, -3, -2, -2, 0, 0, 1, 2]
            prev = {}
            for s in range(FS):
                r = _rows(base + s * HC, HC, HC)
                nrow = HC // 2 + c * (FS * HC // 2) + (s + 1) * (HC // 2)
                if s == FS - 1:
                    nrow = jnp.minimum(nrow, (S - HC) // 2)
                slabs = [None] * 8
                for i in range(8):
                    if REL[i] < 0:
                        slabs[i] = norm_slab(nrow + i * 8, prev.get(NT7 + REL[i]))
                cur = {}
                for n in range(NT7):
                    t = z2_tile(xn, r, n)
                    if n < NT7 - 1:
                        cur[n] = _token(t)
                    for i in range(8):
                        if REL[i] == n:
                            slabs[i] = norm_slab(nrow + i * 8, cur[n])
                prev = cur
                xn = jnp.concatenate(slabs, axis=0)
            nxt_ref[...] = _u32(xn)

        def front1(c):
            pace = {0: [0, 1], 1: [2, 3], 2: [4], 3: [5], 4: [6], 5: [7]}
            for s in range(CH // HC):
                r2 = _rows(c * (CH // 2) + s * (HC // 2), HC // 2, HC // 2)
                xu = xn_ref[r2, :]
                xn = _bf(_after(xu, _token(xu)))
                for n in range(NT7):
                    n0, n1 = n * 128, min((n + 1) * 128, Fh)
                    t = _dot_nt(xn, _bf(winT_ref[n0 // 2:n1 // 2, :]))
                    z1_ref[r2, n0:n1] = _u32(_gelu(t).astype(BF16))
                    for i in pace.get(n, []):
                        off = s * HC + i * 16
                        z2_ref[_rows(c * (CH // 2) + off // 2, 8, 8), :] = _u32(
                            _ln(_after(tmp_ref[_rows(c * CH + off, 16, 16), :], _token(t)), Fh).astype(BF16))

        def gate_rows(half_start, n, align, slot):
            r = _rows(half_start * 2, n, align)
            r2 = _rows(half_start, n // 2, align // 2)
            us = []
            lst_ref[slot, 0:n // 2, :] = wsp_ref[r2, :]

            def part(n0, n1):
                g = _dot(_bf(lst_ref[slot, 0:n // 2, :]), _bf(z2_ref[:, n0:n1]))
                bfull = jnp.concatenate([bcol_ref[r, :]] * (-(-(n1 - n0) // 128)), axis=1)[:, :n1 - n0]
                z1 = _bf(z1_ref[r2, n0:n1]).astype(F32)
                us.append((z1 * g + z1 * bfull).astype(BF16))

            def fin():
                y = _dot(jnp.concatenate(us, axis=1), _bf(wout_ref[...]))
                gate_ref[r, :] = y * (1.0 / (1.0 + jnp.exp(-y)))
            return part, fin

        def relayout(k):
            G = 16
            for i in range(3 * PG):
                sa = k * (6 * PG) + 2 * i
                for q in range(0, D2, G):
                    a = w_ref[sa, q:q + G, :]
                    b = w_ref[sa + 1, q:q + G, :]
                    w_ref[sa, q:q + G, :] = (a & U32(0xFFFF)) | (b << 16)
                    w_ref[sa + 1, q:q + G, :] = (a >> 16) | (b & U32(0xFFFF0000))

        def upfront(c):
            wait_w(c)
            fs = [gate_rows(c * (UC // 2) + i * 32, 64, 64, i) for i in range(UC // 64)]
            for part, _ in fs:
                part(0, Fh)
            for _, fin in fs:
                fin()
            relayout(c)

        cp_x(0).wait()
        xn0 = jnp.concatenate([norm_slab(i * 8) for i in range(8)], axis=0)
        nxt_ref[...] = _u32(jnp.concatenate([norm_slab(HC // 2 + i * 8) for i in range(8)], axis=0))
        cp_b.wait()
        cp_m.wait()
        bT = jnp.concatenate([b_ref[...].astype(F32), jnp.zeros((128 - S // 128, 128), F32)], axis=0).T
        for i in range(S // 128):
            bcol_ref[i * 128:(i + 1) * 128, :] = jnp.broadcast_to(bT[:, i:i + 1], (128, 128))
        mem_ref[...] = mem0_ref[...].astype(F32)
        cp_w2.wait()
        for n in range(NT7):
            z2_tile(xn0, pl.ds(0, HC), n)

        loop(FI, front2)
        for p in range(NW0, NP):
            start_w(p)
        cp_wo.start()
        cp_ws1.start()
        cp_w1.wait()
        loop(NCH, front1)
        cp_wout.wait()
        cp_ws0.wait()
        loop(NU, upfront)
        cp_wo.wait()

        ri = lax.broadcasted_iota(jnp.int32, (2 * L, 2 * L), 0)
        ci = lax.broadcasted_iota(jnp.int32, (2 * L, 2 * L), 1)
        rh = ri >= L
        ch = ci >= L
        rr = jnp.where(rh, ri - L, ri)
        cc = jnp.where(ch, ci - L, ci)
        same = rh == ch
        valid = same & ((rr >= SEG) | (cc >= SEG) | (rr >= cc))
        fill = jnp.where(same, -1e9 / scale, -jnp.inf).astype(F32)

        def heads(t):
            return tuple(
                jnp.concatenate([t[:, (2 * j) * Dh:(2 * j + 1) * Dh], t[:, (2 * j + 1) * Dh:(2 * j + 2) * Dh]],
                                axis=0).astype(BF16) for j in range(3))

        def wpair(p):
            return _bf(jnp.concatenate([w_ref[6 * p + i] for i in range(6)], axis=1))

        def segment(proj, wo_lhs, lag, extra, wo_groups):
            qkv, pm, oc, acc = {}, {}, {}, []

            def score(p):
                q2, k2, _ = qkv[p]
                sc = jnp.where(valid, _dot_nt(q2, k2), fill)
                mx = jnp.max(sc, axis=-1, keepdims=True)
                e = jnp.exp2((sc - mx) * (scale * math.log2(math.e)))
                den = jnp.sum(e, axis=-1, keepdims=True)
                inv = pl.reciprocal(den, approx=True)
                inv = inv * (2.0 - den * inv)
                pm[p] = (e * inv).astype(BF16)

            def pv(p):
                o2 = _dot(pm[p], qkv[p][2])
                oc[p] = jnp.concatenate([o2[:L], o2[L:]], axis=1)

            def wo(ps):
                lhs = jnp.concatenate([wo_lhs(p, oc[p]) for p in ps], axis=1).astype(BF16)
                t = _dot(lhs, _bf(wo_ref[ps[0] * Dh:(ps[-1] + 1) * Dh, :]))
                acc[:] = [t + acc[0] if acc else t]

            fillers = extra + [functools.partial(wo, ps) for ps in wo_groups]
            for i in range(NP + lag):
                if i < NP:
                    qkv[i] = heads(proj(i))
                else:
                    fillers.pop(0)()
                if 1 <= i <= NP:
                    score(i - 1)
                if i >= lag:
                    pv(i - lag)
            for f in fillers:
                f()
            return acc[0], oc

        def pair_step(it, mem_a, slot):
            r = _rows(it * (2 * SEG), 2 * SEG, 2 * SEG)
            gpart, gfin = gate_rows(UP // 2 + it * (BR // 2), BR, 16, slot)
            GS = 256 if slot else 0
            if GS:
                gpart(0, GS)
            xst_ref[slot] = xn_ref[_rows(it * SEG, SEG, SEG), :]
            xs = _bf(xst_ref[slot])
            xb = xs[SEG:].astype(F32)
            ha = jnp.concatenate([xs[:SEG], jnp.concatenate([xb[:M], mem_a], axis=0).astype(BF16)], axis=0)
            early = {}

            def proj_a(p):
                t = _dot(ha, wpair(p))
                early[p] = t[SEG:SEG + M]
                return jnp.concatenate([t[:SEG], t[SEG + M:]], axis=0)

            acc_a, oca = segment(
                proj_a, lambda p, o: jnp.concatenate([o[:SEG - M], o[SEG:]], axis=0), 3, [],
                ([0, 1, 2], [3, 4, 5], [6, 7, 8, 9], [10, 11, 12, 13, 14], [15]))
            mem_b = acc_a[SEG - M:].astype(BF16).astype(F32)
            gpart(GS, Fh)
            hb = jnp.concatenate([xb[M:], mem_b], axis=0).astype(BF16)
            acc_b, _ = segment(
                lambda p: jnp.concatenate([early[p], _dot(hb, wpair(p))], axis=0),
                lambda p, o: jnp.concatenate([oca[p][SEG - M:SEG], o], axis=0), 4, [gfin],
                ([0, 1, 2], [3, 4, 5], [6, 7, 8], [9, 10], [11, 12], [13, 14], [15]))
            sa = jnp.concatenate([acc_a[:SEG - M], acc_b[:SEG + M]], axis=0)
            o_ref[r, :] = (x_ref[r, :].astype(F32) + sa * gate_ref[r, :]).astype(BF16)
            return acc_b[SEG + M:].astype(BF16).astype(F32)

        def step(it):
            @pl.when(it == 1)
            def _():
                cp_ws1.wait()
            mem = mem_ref[...]
            for u in range(UNR):
                mem = pair_step(it * UNR + u, mem, u)
            mem_ref[...] = mem
            r = _rows(it * (UNR * 2 * SEG), UNR * 2 * SEG, 2 * SEG)
            pltpu.make_async_copy(o_ref.at[r, :], o_hbm.at[r, :], osem).start()

        loop(NIT // UNR, step)
        pltpu.make_async_copy(o_ref, o_hbm, osem).wait()

    any_spec = pl.BlockSpec(memory_space=pl.ANY)
    out = pl.pallas_call(
        kern,
        out_shape=jax.ShapeDtypeStruct((S, D), BF16),
        in_specs=[any_spec] * 10,
        out_specs=any_spec,
        scratch_shapes=[
            pltpu.VMEM((S, D), BF16),
            pltpu.VMEM((F // 2, D), U32),
            pltpu.VMEM((3 * H, D2, Dh), U32),
            pltpu.VMEM((H * Dh // 2, D), U32),
            pltpu.VMEM((Fh // 2, D), U32),
            pltpu.VMEM((S // 2, S), U32),
            pltpu.VMEM((S, D), BF16),
            pltpu.VMEM((S // 2, D), U32),
            pltpu.VMEM((S // 2, Fh), U32),
            pltpu.VMEM((S // 2, Fh), U32),
            pltpu.VMEM((S, 128), F32),
            pltpu.VMEM((M, D), F32),
            pltpu.VMEM((S, D), F32),
            pltpu.VMEM((S, Fh), F32),
            pltpu.VMEM((HC // 2, D), U32),
            pltpu.VMEM((max(UNR, UC // 64), 32, S), U32),
            pltpu.VMEM((UNR, SEG, D), U32),
            pltpu.VMEM((M, D), BF16),
            pltpu.VMEM((S // 128, 128), BF16),
            pltpu.SemaphoreType.DMA((FI + 1,)),
            pltpu.SemaphoreType.DMA((NU,)),
            pltpu.SemaphoreType.DMA((8,)),
            pltpu.SemaphoreType.DMA,
        ],
        compiler_params=pltpu.CompilerParams(vmem_limit_bytes=120 * 1024 * 1024),
    )(x2, mem0, wq, wk, wv, wo, winT, B_w_sp, b2, B_w_out)
    return out.reshape(1, S, D)


def pallas_recurrent_scan__memory_aug_recurrent_mem_tr__mixer_gmlp__prompt_kernel(A_x, A_mem0, A_Wq, A_Wk, A_Wv, A_Wo, A_seg_len, B_x, B_w_in, B_w_sp, B_b_sp, B_w_out):
    del B_x
    seg = A_seg_len if isinstance(A_seg_len, int) else 32
    return _run(A_x, A_mem0, A_Wq, A_Wk, A_Wv, A_Wo, B_w_in, B_w_sp, B_b_sp, B_w_out, SEG=seg)
```

```python
import functools
import math

import jax
import jax.numpy as jnp
from jax import lax
import jax.experimental.pallas as pl
import jax.experimental.pallas.tpu as pltpu

F32 = jnp.float32
BF16 = jnp.bfloat16
U32 = jnp.uint32
NT = (((1,), (1,)), ((), ()))
EPS = 1e-5


def _gelu(x):
    c = math.sqrt(2.0 / math.pi)
    h = 0.5 * x
    return h + h * jnp.tanh(x * (c + (c * 0.044715) * (x * x)))


def _dot(a, b):
    return jnp.dot(a, b, preferred_element_type=F32)


def _dot_nt(a, b):
    return lax.dot_general(a, b, NT, preferred_element_type=F32)


def _bf(u32_val):
    return pltpu.bitcast(u32_val, BF16)


def _u32(bf_val):
    return pltpu.bitcast(bf_val, U32)


def _token(t):
    b = pltpu.bitcast(t[0:8, 0:128], U32)
    return (b >> 16) >> 16


def _after(x, tok):
    if tok is None:
        return x
    r, c = x.shape
    z = jnp.concatenate([tok] * (r // 8), axis=0)
    z = jnp.concatenate([z] * (c // 128), axis=1)
    return pltpu.bitcast(pltpu.bitcast(x, U32) | z, x.dtype)


def _rows(start, size, align):
    return pl.ds(pl.multiple_of(start, align), size)


@functools.partial(jax.jit, static_argnames=("SEG",))
def _run(A_x, A_mem0, A_Wq, A_Wk, A_Wv, A_Wo, B_w_in, B_w_sp, B_b_sp, B_w_out, *, SEG):
    _, S, D = A_x.shape
    H, Dh = A_Wq.shape[1], A_Wq.shape[2]
    M = A_mem0.shape[1]
    F = B_w_in.shape[1]
    assert (S, D, H, Dh, M, SEG, F) == (2048, 640, 32, 128, 8, 32, 1728) and A_x.shape[0] == 1
    L = SEG + M
    Fh = F // 2
    HF = Fh // 2
    scale = Dh ** -0.5
    NP = H // 2
    D2 = D // 2
    TB = 4 * SEG
    HB = TB // 2
    NB = S // TB
    RC = 144
    NRC = Fh // RC
    FS = 5
    FI = (NB - 1) // FS
    Z1B = 8
    FU = 512
    GB = 4
    NU = NB // GB
    PG = NP // NU

    x2 = A_x.reshape(S, D)
    mem0 = A_mem0.reshape(M, D)
    wq = A_Wq.reshape(D2, 2 * H, Dh)
    wk = A_Wk.reshape(D2, 2 * H, Dh)
    wv = A_Wv.reshape(D2, 2 * H, Dh)
    wo = A_Wo.reshape(H * Dh, D)
    winT = B_w_in.T
    b2 = B_b_sp.reshape(NB, TB)

    def kern(x_hbm, mem0_hbm, wq_hbm, wk_hbm, wv_hbm, wo_hbm, winT_hbm, wsp_hbm, b_hbm, wout_hbm,
             o_hbm,
             x_ref, winT_ref, w_ref, wo_ref, wout_ref, wsp_ref, o_ref,
             xn_ref, z_ref, brow_ref, mem_ref, u_ref, tmp_ref, nxt_ref, lst_ref, xst_ref,
             mem0_ref, b_ref, qst_ref, xsem, wsem, ssem, sem, osem):
        w_hbm = [w.bitcast(U32) for w in (wq_hbm, wk_hbm, wv_hbm)]
        wsp32 = wsp_hbm.bitcast(U32)
        winT32 = winT_hbm.bitcast(U32)

        XB = [0, 2 * TB] + [min(2 * TB + (c + 1) * FS * TB, S) for c in range(FI)]

        def cp_x(c):
            return pltpu.make_async_copy(x_hbm.at[XB[c]:XB[c + 1], :], x_ref.at[XB[c]:XB[c + 1], :], xsem.at[c])

        def cp_ws(k):
            r2 = pl.ds(k * (GB * HB), GB * HB)
            return pltpu.make_async_copy(wsp32.at[r2], wsp_ref.at[r2], ssem.at[k])

        def start_group(k):
            cp_ws(k).start()
            for p in range(k * PG, (k + 1) * PG):
                for j in range(3):
                    for par in range(2):
                        pltpu.make_async_copy(w_hbm[j].at[:, par * NP + p, :],
                                              w_ref.at[6 * p + 2 * j + par], wsem.at[k]).start()

        def wait_group(k):
            cp_ws(k).wait()
            grp = w_ref.at[pl.ds(k * (6 * PG), 6 * PG)]
            pltpu.make_async_copy(grp, grp, wsem.at[k]).wait()

        cp_w2 = pltpu.make_async_copy(winT32.at[HF:], winT_ref.at[HF:], sem.at[0])
        cp_w1 = pltpu.make_async_copy(winT32.at[:HF], winT_ref.at[:HF], sem.at[1])
        cp_wo = pltpu.make_async_copy(wo_hbm.bitcast(U32), wo_ref, sem.at[2])
        cp_wout = pltpu.make_async_copy(wout_hbm.bitcast(U32), wout_ref, sem.at[3])
        cp_m = pltpu.make_async_copy(mem0_hbm, mem0_ref, sem.at[4])
        cp_b = pltpu.make_async_copy(b_hbm, b_ref, sem.at[5])

        cp_x(0).start()
        cp_b.start()
        cp_m.start()
        cp_w2.start()
        for c in range(1, FI + 1):
            cp_x(c).start()
        cp_w1.start()
        start_group(0)
        start_group(1)

        def loop(n, fn):
            def body(c, carry):
                fn(c)
                return carry
            lax.fori_loop(0, n, body, 0)

        def norm_slab(hrow, srow, tok=None):
            x = _after(x_ref[_rows(hrow * 2, 16, 16), :].astype(F32), tok)
            d = x - jnp.sum(x, axis=-1, keepdims=True) * (1.0 / D)
            xn = d * lax.rsqrt(jnp.sum(d * d, axis=-1, keepdims=True) * (1.0 / D) + EPS)
            xu = _u32(xn.astype(BF16))
            xn_ref[_rows(hrow, 8, 8), 0:D] = xu
            nxt_ref[srow:srow + 8, 0:D] = xu

        def z2_chunk(xn, j, n):
            t = _dot_nt(_bf(winT_ref[HF + n * RC // 2:HF + (n + 1) * RC // 2, :]), xn)
            tmp_ref[j, n * RC:(n + 1) * RC, :] = _gelu(t)
            return t

        def front2(c):
            for k in range(FI):
                @pl.when(c == k)
                def _():
                    cp_x(k + 1).wait()
            rel = [-2, -2, -1, -1, 0, 0, 1, 2]
            prev = {}
            for s in range(FS):
                j = 1 + c * FS + s
                nrow = (j + 1) * HB
                if s == FS - 1:
                    nrow = jnp.minimum(nrow, (NB - 1) * HB)
                xn = _bf(nxt_ref[s * HB:(s + 1) * HB, 0:D])
                srow = ((s + 1) % FS) * HB
                for i in range(8):
                    if rel[i] < 0:
                        norm_slab(nrow + i * 8, srow + i * 8, prev.get(NRC + rel[i]))
                cur = {}
                for n in range(NRC):
                    cur[n] = _token(z2_chunk(xn, j, n))
                    for i in range(8):
                        if rel[i] == n:
                            norm_slab(nrow + i * 8, srow + i * 8, cur[n])
                prev = cur

        def ln_block(j, tok):
            G = 48
            rep = lambda v: jnp.concatenate([v] * (G // 8), axis=0)
            acc = pltpu.bitcast(tok, F32)
            for q in range(0, Fh, 8):
                acc = acc + tmp_ref[j, q:q + 8, :]
            mean = jnp.broadcast_to(jnp.sum(acc, axis=0, keepdims=True) * (1.0 / Fh), (8, TB))
            acc = None
            for q in range(0, Fh, G):
                m = mean if acc is None else _after(mean, _token(acc))
                d = tmp_ref[j, q:q + G, :] - rep(m)
                part = jnp.sum((d * d).reshape(G // 8, 8, TB), axis=0)
                acc = part if acc is None else acc + part
            rstd = lax.rsqrt(jnp.sum(acc, axis=0, keepdims=True) * (1.0 / Fh) + EPS)
            tok = _token(jnp.broadcast_to(rstd, (8, TB)))
            for q in range(0, Fh, G):
                o = (tmp_ref[j, q:q + G, :] - rep(_after(mean, tok))) * rstd
                z_ref[_rows(j * HF + q // 2, G // 2, 8), TB:2 * TB] = _u32(o.astype(BF16))
                tok = _token(o)

        def front1(c):
            tok = None
            for s in range(Z1B):
                j = c * Z1B + s
                xu = xn_ref[_rows(j * HB, HB, HB), 0:D]
                if tok is None:
                    tok = _token(xu)
                    ln_block(j, tok)
                xn = _bf(_after(xu, tok))
                for n in range(NRC):
                    t = _dot_nt(_bf(winT_ref[n * RC // 2:(n + 1) * RC // 2, :]), xn)
                    z_ref[_rows(j * HF + n * RC // 2, RC // 2, 8), 0:TB] = _u32(_gelu(t).astype(BF16))
                    if n == 2:
                        tok = _token(t)
                    if n == 3 and s + 1 < Z1B:
                        ln_block(j + 1, _token(t))

        def stage_ws(j, slot):
            lst_ref[slot] = wsp_ref[_rows(j * HB, HB, HB), :]

        def ut_part(j, slot, f0, f1, tok=None):
            zs = [z_ref[k * HF + f0 // 2:k * HF + f1 // 2, TB:2 * TB] for k in range(NB)]
            zs[0] = _after(zs[0], tok)
            gt = _dot_nt(_bf(jnp.concatenate(zs, axis=1)), _bf(lst_ref[slot]))
            z1t = _bf(z_ref[_rows(j * HF + f0 // 2, (f1 - f0) // 2, 8), 0:TB]).astype(F32)
            bt = jnp.concatenate([brow_ref[j]] * ((f1 - f0) // 8), axis=0)
            return z1t * gt + z1t * bt

        def untranspose(ut):
            n = ut.shape[0]
            if n < TB:
                ut = jnp.concatenate([ut, jnp.zeros((TB - n, TB), F32)], axis=0)
            return ut.T[:, :n].astype(BF16)

        def relayout(k, tok):
            G = 16
            for i in range(3 * PG):
                sa = k * (6 * PG) + 2 * i
                for q in range(0, D2, G):
                    lo = jnp.concatenate([tok | U32(0xFFFF)] * (G // 8), axis=0)
                    hi = jnp.concatenate([tok | U32(0xFFFF0000)] * (G // 8), axis=0)
                    a = w_ref[sa, q:q + G, :]
                    b = w_ref[sa + 1, q:q + G, :]
                    h0 = (a & lo) | (b << 16)
                    w_ref[sa, q:q + G, :] = h0
                    w_ref[sa + 1, q:q + G, :] = (a >> 16) | (b & hi)
                    tok = _token(h0)

        def upfront(c):
            wait_group(c)
            for s in range(GB):
                j = c * GB + s
                stage_ws(j, s)
                for f0 in range(0, FU, TB):
                    ut = ut_part(j, s, f0, f0 + TB)
                    u_ref[_rows(j * (FU // 2) + f0 // 2, HB, 8), 0:TB] = _u32(ut.astype(BF16))
                    if s == 0 and f0 == 0:
                        relayout(c, _token(ut))

        cp_x(0).wait()
        for i in range(8):
            norm_slab(i * 8, HB + i * 8)
        xn0 = _bf(nxt_ref[HB:2 * HB, 0:D])
        for i in range(8):
            norm_slab(HB + i * 8, i * 8)
        cp_b.wait()
        cp_m.wait()
        bf32 = b_ref[...].astype(F32)
        for i in range(NB):
            brow_ref[i] = jnp.broadcast_to(bf32[i:i + 1, :], (8, TB))
        mem_ref[...] = mem0_ref[...].astype(F32)
        cp_w2.wait()
        for n in range(NRC):
            z2_chunk(xn0, 0, n)

        loop(FI, front2)
        start_group(2)
        cp_w1.wait()
        loop(NB // Z1B, front1)
        start_group(3)
        cp_wout.start()
        cp_wo.start()
        loop(NU, upfront)
        cp_wout.wait()
        cp_wo.wait()

        ri = lax.broadcasted_iota(jnp.int32, (2 * L, 2 * L), 0)
        ci = lax.broadcasted_iota(jnp.int32, (2 * L, 2 * L), 1)
        rh = ri >= L
        ch = ci >= L
        rr = jnp.where(rh, ri - L, ri)
        cc = jnp.where(ch, ci - L, ci)
        same = rh == ch
        valid = same & ((rr >= SEG) | (cc >= SEG) | (rr >= cc))
        fill = jnp.where(same, -1e9 / scale, -jnp.inf).astype(F32)

        def wpair(p):
            return _bf(jnp.concatenate([w_ref[6 * p + i] for i in range(6)], axis=1))

        def segment(proj, wo_lhs, lag, extra, wo_groups):
            pm, oc, acc = {}, {}, []

            def qkv(p, j):
                return _bf(qst_ref[p * L:(p + 1) * L, j * Dh:(j + 1) * Dh])

            def project(p):
                t = proj(p)
                for j in range(3):
                    two = jnp.concatenate([t[:, 2 * j * Dh:(2 * j + 1) * Dh],
                                           t[:, (2 * j + 1) * Dh:(2 * j + 2) * Dh]], axis=0)
                    qst_ref[p * L:(p + 1) * L, j * Dh:(j + 1) * Dh] = _u32(two.astype(BF16))

            def score(p):
                sc = jnp.where(valid, _dot_nt(qkv(p, 0), qkv(p, 1)), fill)
                mx = jnp.max(sc, axis=-1, keepdims=True)
                e = jnp.exp2((sc - mx) * (scale * math.log2(math.e)))
                den = jnp.sum(e, axis=-1, keepdims=True)
                inv = pl.reciprocal(den, approx=True)
                inv = inv * (2.0 - den * inv)
                pm[p] = (e * inv).astype(BF16)

            def pv(p):
                o2 = _dot(pm[p], qkv(p, 2))
                oc[p] = jnp.concatenate([o2[:L], o2[L:]], axis=1)

            def wo(ps):
                lhs = jnp.concatenate([wo_lhs(p, oc[p]) for p in ps], axis=1).astype(BF16)
                t = _dot(lhs, _bf(wo_ref[ps[0] * Dh:(ps[-1] + 1) * Dh, :]))
                acc[:] = [t + acc[0] if acc else t]

            fillers = extra + [functools.partial(wo, ps) for ps in wo_groups]
            for i in range(NP + lag):
                if i < NP:
                    project(i)
                else:
                    fillers.pop(0)()
                if 1 <= i <= NP:
                    score(i - 1)
                if i >= lag:
                    pv(i - lag)
            for f in fillers:
                f()
            return acc[0], oc

        def pair_step(ip, mem_a, slot, fill_a, fill_b, extra):
            fill_a()
            xst_ref[slot] = xn_ref[_rows(ip * SEG, SEG, SEG), 0:D]
            xs = _bf(xst_ref[slot])
            xb = xs[SEG:].astype(F32)
            ha = jnp.concatenate([xs[:SEG], jnp.concatenate([xb[:M], mem_a], axis=0).astype(BF16)], axis=0)
            early = {}

            def proj_a(p):
                t = _dot(ha, wpair(p))
                early[p] = t[SEG:SEG + M]
                return jnp.concatenate([t[:SEG], t[SEG + M:]], axis=0)

            acc_a, oca = segment(
                proj_a, lambda p, o: jnp.concatenate([o[:SEG - M], o[SEG:]], axis=0), 3, [],
                ([0, 1, 2], [3, 4, 5], [6, 7, 8, 9], [10, 11, 12, 13, 14], [15]))
            mem_b = acc_a[SEG - M:].astype(BF16).astype(F32)
            fill_b()
            hb = jnp.concatenate([xb[M:], mem_b], axis=0).astype(BF16)
            acc_b, _ = segment(
                lambda p: jnp.concatenate([early[p], _dot(hb, wpair(p))], axis=0),
                lambda p, o: jnp.concatenate([oca[p][SEG - M:SEG], o], axis=0), 4, extra,
                ([0, 1, 2], [3, 4, 5], [6, 7, 8], [9, 10], [11, 12], [13, 14], [15]))
            sa = jnp.concatenate([acc_a[:SEG - M], acc_b[:SEG + M]], axis=0)
            return sa, acc_b[SEG + M:].astype(BF16).astype(F32)

        def step(it):
            r = _rows(it * TB, TB, TB)
            stage_ws(it, 0)
            us = [untranspose(_bf(u_ref[_rows(it * (FU // 2) + f0 // 2, HB, 8), 0:TB]).astype(F32))
                  for f0 in range(0, FU, TB)]
            gate = []

            def rest(f0):
                toks = [_token(_u32(u)[HB - 8:]) for u in (us if f0 == FU else us[-1:])]
                tok = functools.reduce(lambda a, b: a | b, toks)
                us.append(untranspose(ut_part(it, 0, f0, min(f0 + TB, Fh), tok)))

            def fin():
                y = _dot(jnp.concatenate(us, axis=1), _bf(wout_ref[...]))
                gate.append(y * (1.0 / (1.0 + jnp.exp(-y))))

            s0, mem = pair_step(it * 2, mem_ref[...], 0, lambda: None, lambda: rest(FU), [])
            s1, mem = pair_step(it * 2 + 1, mem, 1, lambda: rest(FU + TB), lambda: rest(FU + 2 * TB), [fin])
            mem_ref[...] = mem
            o_ref[r, :] = (x_ref[r, :].astype(F32) + jnp.concatenate([s0, s1], axis=0) * gate[0]).astype(BF16)
            pltpu.make_async_copy(o_ref.at[r, :], o_hbm.at[r, :], osem).start()

        loop(NB, step)
        pltpu.make_async_copy(o_ref, o_hbm, osem).wait()

    any_spec = pl.BlockSpec(memory_space=pl.ANY)
    out = pl.pallas_call(
        kern,
        out_shape=jax.ShapeDtypeStruct((S, D), BF16),
        in_specs=[any_spec] * 10,
        out_specs=any_spec,
        scratch_shapes=[
            pltpu.VMEM((S, D), BF16),
            pltpu.VMEM((F // 2, D), U32),
            pltpu.VMEM((3 * H, D2, Dh), U32),
            pltpu.VMEM((H * Dh // 2, D), U32),
            pltpu.VMEM((HF, D), U32),
            pltpu.VMEM((S // 2, S), U32),
            pltpu.VMEM((S, D), BF16),
            pltpu.VMEM((S // 2, D + 128), U32),
            pltpu.VMEM((NB * HF, 2 * TB), U32),
            pltpu.VMEM((NB, 8, TB), F32),
            pltpu.VMEM((M, D), F32),
            pltpu.VMEM((NB * FU // 2, 2 * TB), U32),
            pltpu.VMEM((NB, Fh, TB), F32),
            pltpu.VMEM((FS * HB, D + 128), U32),
            pltpu.VMEM((GB, HB, S), U32),
            pltpu.VMEM((2, SEG, D), U32),
            pltpu.VMEM((M, D), BF16),
            pltpu.VMEM((NB, TB), BF16),
            pltpu.VMEM((NP * L, 3 * Dh), U32),
            pltpu.SemaphoreType.DMA((FI + 1,)),
            pltpu.SemaphoreType.DMA((NU,)),
            pltpu.SemaphoreType.DMA((NU,)),
            pltpu.SemaphoreType.DMA((6,)),
            pltpu.SemaphoreType.DMA,
        ],
        compiler_params=pltpu.CompilerParams(vmem_limit_bytes=120 * 1024 * 1024),
    )(x2, mem0, wq, wk, wv, wo, winT, B_w_sp, b2, B_w_out)
    return out.reshape(1, S, D)


def pallas_recurrent_scan__memory_aug_recurrent_mem_tr__mixer_gmlp__prompt_kernel(A_x, A_mem0, A_Wq, A_Wk, A_Wv, A_Wo, A_seg_len, B_x, B_w_in, B_w_sp, B_b_sp, B_w_out):
    del B_x
    seg = A_seg_len if isinstance(A_seg_len, int) else 32
    return _run(A_x, A_mem0, A_Wq, A_Wk, A_Wv, A_Wo, B_w_in, B_w_sp, B_b_sp, B_w_out, SEG=seg)
```

```python
import functools
import math

import jax
import jax.numpy as jnp
from jax import lax
import jax.experimental.pallas as pl
import jax.experimental.pallas.tpu as pltpu

F32 = jnp.float32
BF16 = jnp.bfloat16
U32 = jnp.uint32
NT = (((1,), (1,)), ((), ()))
EPS = 1e-5


def _gelu(x):
    c = math.sqrt(2.0 / math.pi)
    h = 0.5 * x
    return h + h * jnp.tanh(x * (c + (c * 0.044715) * (x * x)))


def _dot(a, b):
    return jnp.dot(a, b, preferred_element_type=F32)


def _dot_nt(a, b):
    return lax.dot_general(a, b, NT, preferred_element_type=F32)


def _bf(u32_val):
    return pltpu.bitcast(u32_val, BF16)


def _u32(bf_val):
    return pltpu.bitcast(bf_val, U32)


def _token(t):
    b = pltpu.bitcast(t[0:8, 0:128], U32)
    return (b >> 16) >> 16


def _after(x, tok):
    if tok is None:
        return x
    r, c = x.shape
    z = jnp.concatenate([tok] * (r // 8), axis=0)
    z = jnp.concatenate([z] * (c // 128), axis=1)
    return pltpu.bitcast(pltpu.bitcast(x, U32) | z, x.dtype)


def _rows(start, size, align):
    return pl.ds(pl.multiple_of(start, align), size)


@functools.partial(jax.jit, static_argnames=("SEG",))
def _run(A_x, A_mem0, A_Wq, A_Wk, A_Wv, A_Wo, B_w_in, B_w_sp, B_b_sp, B_w_out, *, SEG):
    _, S, D = A_x.shape
    H, Dh = A_Wq.shape[1], A_Wq.shape[2]
    M = A_mem0.shape[1]
    F = B_w_in.shape[1]
    assert (S, D, H, Dh, M, SEG, F) == (2048, 640, 32, 128, 8, 32, 1728) and A_x.shape[0] == 1
    L = SEG + M
    Fh = F // 2
    HF = Fh // 2
    scale = Dh ** -0.5
    NP = H // 2
    D2 = D // 2
    TB = 4 * SEG
    HB = TB // 2
    NB = S // TB
    RC = 144
    NRC = Fh // RC
    PK = 4
    C0 = 2
    FS = 6
    FI = (NB - PK) // FS
    Z1B = 8
    FU = 512
    GB = 4
    NU = NB // GB
    PG = NP // NU

    x2 = A_x.reshape(S, D)
    mem0 = A_mem0.reshape(M, D)
    wq = A_Wq.reshape(D2, 2 * H, Dh)
    wk = A_Wk.reshape(D2, 2 * H, Dh)
    wv = A_Wv.reshape(D2, 2 * H, Dh)
    wo = A_Wo.reshape(H * Dh, D)
    winT = B_w_in.T
    b2 = B_b_sp.reshape(NB, TB)

    def kern(x_hbm, mem0_hbm, wq_hbm, wk_hbm, wv_hbm, wo_hbm, winT_hbm, wsp_hbm, b_hbm, wout_hbm,
             o_hbm,
             x_ref, winT_ref, w_ref, wo_ref, wout_ref, wsp_ref, o_ref,
             xn_ref, z_ref, brow_ref, mem_ref, u_ref, tmp_ref, nxt_ref, lst_ref, xst_ref,
             mem0_ref, b_ref, qst_ref, xsem, wsem, ssem, sem, osem):
        w_hbm = [w.bitcast(U32) for w in (wq_hbm, wk_hbm, wv_hbm)]
        wsp32 = wsp_hbm.bitcast(U32)
        winT32 = winT_hbm.bitcast(U32)

        XB = [0, PK * TB, (PK + 1) * TB] + [min((PK + 1 + (c + 1) * FS) * TB, S) for c in range(FI)]

        def cp_x(c):
            return pltpu.make_async_copy(x_hbm.at[XB[c]:XB[c + 1], :], x_ref.at[XB[c]:XB[c + 1], :], xsem.at[c])

        def cp_ws(k):
            r2 = pl.ds(k * (GB * HB), GB * HB)
            return pltpu.make_async_copy(wsp32.at[r2], wsp_ref.at[r2], ssem.at[k])

        def start_group(k):
            cp_ws(k).start()
            for p in range(k * PG, (k + 1) * PG):
                for j in range(3):
                    for par in range(2):
                        pltpu.make_async_copy(w_hbm[j].at[:, par * NP + p, :],
                                              w_ref.at[6 * p + 2 * j + par], wsem.at[k]).start()

        def wait_group(k):
            cp_ws(k).wait()
            grp = w_ref.at[pl.ds(k * (6 * PG), 6 * PG)]
            pltpu.make_async_copy(grp, grp, wsem.at[k]).wait()

        WA = HF + C0 * RC // 2
        cp_w2a = pltpu.make_async_copy(winT32.at[HF:WA], winT_ref.at[HF:WA], sem.at[0])
        cp_w2b = pltpu.make_async_copy(winT32.at[WA:], winT_ref.at[WA:], sem.at[6])
        cp_w1 = pltpu.make_async_copy(winT32.at[:HF], winT_ref.at[:HF], sem.at[1])
        cp_wo = pltpu.make_async_copy(wo_hbm.bitcast(U32), wo_ref, sem.at[2])
        cp_wout = pltpu.make_async_copy(wout_hbm.bitcast(U32), wout_ref, sem.at[3])
        cp_m = pltpu.make_async_copy(mem0_hbm, mem0_ref, sem.at[4])
        cp_b = pltpu.make_async_copy(b_hbm, b_ref, sem.at[5])

        cp_x(0).start()
        cp_w2a.start()
        cp_w2b.start()
        for c in range(1, FI + 2):
            cp_x(c).start()
        cp_b.start()
        cp_m.start()
        cp_w1.start()
        start_group(0)
        start_group(1)

        def loop(n, fn):
            def body(c, carry):
                fn(c)
                return carry
            lax.fori_loop(0, n, body, 0)

        def norm_slab(hrow, srow, tok=None):
            x = _after(x_ref[_rows(hrow * 2, 16, 16), :].astype(F32), tok)
            d = x - jnp.sum(x, axis=-1, keepdims=True) * (1.0 / D)
            xn = d * lax.rsqrt(jnp.sum(d * d, axis=-1, keepdims=True) * (1.0 / D) + EPS)
            xu = _u32(xn.astype(BF16))
            xn_ref[_rows(hrow, 8, 8), 0:D] = xu
            nxt_ref[srow:srow + 8, 0:D] = xu

        def z2_chunk(xn, j, n):
            t = _dot_nt(_bf(winT_ref[HF + n * RC // 2:HF + (n + 1) * RC // 2, :]), xn)
            tmp_ref[j, n * RC:(n + 1) * RC, :] = _gelu(t)
            return t

        def front2(c):
            for k in range(FI):
                @pl.when(c == k)
                def _():
                    cp_x(k + 2).wait()
            rel = [-2, -2, -1, -1, 0, 0, 1, 2]
            prev = {}
            for s in range(FS):
                j = PK + c * FS + s
                nrow = (j + 1) * HB
                if s == FS - 1:
                    nrow = jnp.minimum(nrow, (NB - 1) * HB)
                xn = _bf(nxt_ref[s * HB:(s + 1) * HB, 0:D])
                srow = ((s + 1) % FS) * HB
                for i in range(8):
                    if rel[i] < 0:
                        norm_slab(nrow + i * 8, srow + i * 8, prev.get(NRC + rel[i]))
                cur = {}
                for n in range(NRC):
                    cur[n] = _token(z2_chunk(xn, j, n))
                    for i in range(8):
                        if rel[i] == n:
                            norm_slab(nrow + i * 8, srow + i * 8, cur[n])
                prev = cur

        def ln_block(j, tok):
            G = 48
            rep = lambda v: jnp.concatenate([v] * (G // 8), axis=0)
            acc = pltpu.bitcast(tok, F32)
            for q in range(0, Fh, 8):
                acc = acc + tmp_ref[j, q:q + 8, :]
            mean = jnp.broadcast_to(jnp.sum(acc, axis=0, keepdims=True) * (1.0 / Fh), (8, TB))
            acc = None
            for q in range(0, Fh, G):
                m = mean if acc is None else _after(mean, _token(acc))
                d = tmp_ref[j, q:q + G, :] - rep(m)
                part = jnp.sum((d * d).reshape(G // 8, 8, TB), axis=0)
                acc = part if acc is None else acc + part
            rstd = lax.rsqrt(jnp.sum(acc, axis=0, keepdims=True) * (1.0 / Fh) + EPS)
            tok = _token(jnp.broadcast_to(rstd, (8, TB)))
            for q in range(0, Fh, G):
                o = (tmp_ref[j, q:q + G, :] - rep(_after(mean, tok))) * rstd
                z_ref[_rows(j * HF + q // 2, G // 2, 8), TB:2 * TB] = _u32(o.astype(BF16))
                tok = _token(o)

        def front1(c):
            tok = None
            for s in range(Z1B):
                j = c * Z1B + s
                xu = xn_ref[_rows(j * HB, HB, HB), 0:D]
                if tok is None:
                    tok = _token(xu)
                    ln_block(j, tok)
                xn = _bf(_after(xu, tok))
                for n in range(NRC):
                    t = _dot_nt(_bf(winT_ref[n * RC // 2:(n + 1) * RC // 2, :]), xn)
                    z_ref[_rows(j * HF + n * RC // 2, RC // 2, 8), 0:TB] = _u32(_gelu(t).astype(BF16))
                    if n == 2:
                        tok = _token(t)
                    if n == 3 and s + 1 < Z1B:
                        ln_block(j + 1, _token(t))

        def stage_ws(j, slot):
            lst_ref[slot] = wsp_ref[_rows(j * HB, HB, HB), :]

        def ut_part(j, slot, f0, f1, tok=None):
            zs = [z_ref[k * HF + f0 // 2:k * HF + f1 // 2, TB:2 * TB] for k in range(NB)]
            zs[0] = _after(zs[0], tok)
            gt = _dot_nt(_bf(jnp.concatenate(zs, axis=1)), _bf(lst_ref[slot]))
            z1t = _bf(z_ref[_rows(j * HF + f0 // 2, (f1 - f0) // 2, 8), 0:TB]).astype(F32)
            bt = jnp.concatenate([brow_ref[j]] * ((f1 - f0) // 8), axis=0)
            return z1t * gt + z1t * bt

        def untranspose(ut):
            n = ut.shape[0]
            if n < TB:
                ut = jnp.concatenate([ut, jnp.zeros((TB - n, TB), F32)], axis=0)
            return ut.T[:, :n].astype(BF16)

        def relayout(k, tok):
            G = 16
            for i in range(3 * PG):
                sa = k * (6 * PG) + 2 * i
                for q in range(0, D2, G):
                    lo = jnp.concatenate([tok | U32(0xFFFF)] * (G // 8), axis=0)
                    hi = jnp.concatenate([tok | U32(0xFFFF0000)] * (G // 8), axis=0)
                    a = w_ref[sa, q:q + G, :]
                    b = w_ref[sa + 1, q:q + G, :]
                    h0 = (a & lo) | (b << 16)
                    w_ref[sa, q:q + G, :] = h0
                    w_ref[sa + 1, q:q + G, :] = (a >> 16) | (b & hi)
                    tok = _token(h0)

        def upfront(c):
            wait_group(c)
            for s in range(GB):
                j = c * GB + s
                stage_ws(j, s)
                for f0 in range(0, FU, TB):
                    ut = ut_part(j, s, f0, f0 + TB)
                    u_ref[_rows(j * (FU // 2) + f0 // 2, HB, 8), 0:TB] = _u32(ut.astype(BF16))
                    if s == 0 and f0 == 0:
                        relayout(c, _token(ut))

        cp_x(0).wait()
        for i in range(16):
            norm_slab(i * 8, HB + i * 8)
        cp_w2a.wait()
        for i in range(16, 8 * PK):
            norm_slab(i * 8, HB + i * 8)
        for j in range(PK):
            for n in range(C0):
                z2_chunk(_bf(nxt_ref[(j + 1) * HB:(j + 2) * HB, 0:D]), j, n)
        cp_w2b.wait()
        cp_x(1).wait()
        i = 0
        for j in range(PK):
            for n in range(C0, NRC):
                t = z2_chunk(_bf(nxt_ref[(j + 1) * HB:(j + 2) * HB, 0:D]), j, n)
                if i < 8:
                    norm_slab(PK * HB + i * 8, i * 8, _token(t))
                    i += 1

        loop(FI, front2)
        start_group(2)
        cp_b.wait()
        cp_m.wait()
        bf32 = b_ref[...].astype(F32)
        for i in range(NB):
            brow_ref[i] = jnp.broadcast_to(bf32[i:i + 1, :], (8, TB))
        mem_ref[...] = mem0_ref[...].astype(F32)
        cp_w1.wait()
        loop(NB // Z1B, front1)
        start_group(3)
        cp_wout.start()
        cp_wo.start()
        loop(NU, upfront)
        cp_wout.wait()
        cp_wo.wait()

        ri = lax.broadcasted_iota(jnp.int32, (2 * L, 2 * L), 0)
        ci = lax.broadcasted_iota(jnp.int32, (2 * L, 2 * L), 1)
        rh = ri >= L
        ch = ci >= L
        rr = jnp.where(rh, ri - L, ri)
        cc = jnp.where(ch, ci - L, ci)
        same = rh == ch
        valid = same & ((rr >= SEG) | (cc >= SEG) | (rr >= cc))
        fill = jnp.where(same, -1e9 / scale, -jnp.inf).astype(F32)

        def wpair(p):
            return _bf(jnp.concatenate([w_ref[6 * p + i] for i in range(6)], axis=1))

        def segment(proj, wo_lhs, lag, extra, wo_groups):
            pm, oc, acc = {}, {}, []

            def qkv(p, j):
                return _bf(qst_ref[p * L:(p + 1) * L, j * Dh:(j + 1) * Dh])

            def project(p):
                t = proj(p)
                for j in range(3):
                    two = jnp.concatenate([t[:, 2 * j * Dh:(2 * j + 1) * Dh],
                                           t[:, (2 * j + 1) * Dh:(2 * j + 2) * Dh]], axis=0)
                    qst_ref[p * L:(p + 1) * L, j * Dh:(j + 1) * Dh] = _u32(two.astype(BF16))

            def score(p):
                sc = jnp.where(valid, _dot_nt(qkv(p, 0), qkv(p, 1)), fill)
                mx = jnp.max(sc, axis=-1, keepdims=True)
                e = jnp.exp2((sc - mx) * (scale * math.log2(math.e)))
                den = jnp.sum(e, axis=-1, keepdims=True)
                inv = pl.reciprocal(den, approx=True)
                inv = inv * (2.0 - den * inv)
                pm[p] = (e * inv).astype(BF16)

            def pv(p):
                o2 = _dot(pm[p], qkv(p, 2))
                oc[p] = jnp.concatenate([o2[:L], o2[L:]], axis=1)

            def wo(ps):
                lhs = jnp.concatenate([wo_lhs(p, oc[p]) for p in ps], axis=1).astype(BF16)
                t = _dot(lhs, _bf(wo_ref[ps[0] * Dh:(ps[-1] + 1) * Dh, :]))
                acc[:] = [t + acc[0] if acc else t]

            fillers = extra + [functools.partial(wo, ps) for ps in wo_groups]
            for i in range(NP + lag):
                if i < NP:
                    project(i)
                else:
                    fillers.pop(0)()
                if 1 <= i <= NP:
                    score(i - 1)
                if i >= lag:
                    pv(i - lag)
            for f in fillers:
                f()
            return acc[0], oc

        def pair_step(ip, mem_a, slot, fill_a, fill_b, extra):
            fill_a()
            xst_ref[slot] = xn_ref[_rows(ip * SEG, SEG, SEG), 0:D]
            xs = _bf(xst_ref[slot])
            xb = xs[SEG:].astype(F32)
            ha = jnp.concatenate([xs[:SEG], jnp.concatenate([xb[:M], mem_a], axis=0).astype(BF16)], axis=0)
            early = {}

            def proj_a(p):
                t = _dot(ha, wpair(p))
                early[p] = t[SEG:SEG + M]
                return jnp.concatenate([t[:SEG], t[SEG + M:]], axis=0)

            acc_a, oca = segment(
                proj_a, lambda p, o: jnp.concatenate([o[:SEG - M], o[SEG:]], axis=0), 3, [],
                ([0, 1, 2], [3, 4, 5], [6, 7, 8, 9], [10, 11, 12, 13, 14], [15]))
            mem_b = acc_a[SEG - M:].astype(BF16).astype(F32)
            fill_b()
            hb = jnp.concatenate([xb[M:], mem_b], axis=0).astype(BF16)
            acc_b, _ = segment(
                lambda p: jnp.concatenate([early[p], _dot(hb, wpair(p))], axis=0),
                lambda p, o: jnp.concatenate([oca[p][SEG - M:SEG], o], axis=0), 4, extra,
                ([0, 1, 2], [3, 4, 5], [6, 7, 8], [9, 10], [11, 12], [13, 14], [15]))
            sa = jnp.concatenate([acc_a[:SEG - M], acc_b[:SEG + M]], axis=0)
            return sa, acc_b[SEG + M:].astype(BF16).astype(F32)

        def step(it):
            r = _rows(it * TB, TB, TB)
            stage_ws(it, 0)
            us = [untranspose(_bf(u_ref[_rows(it * (FU // 2) + f0 // 2, HB, 8), 0:TB]).astype(F32))
                  for f0 in range(0, FU, TB)]
            gate = []

            def rest(f0):
                toks = [_token(_u32(u)[HB - 8:]) for u in (us if f0 == FU else us[-1:])]
                tok = functools.reduce(lambda a, b: a | b, toks)
                us.append(untranspose(ut_part(it, 0, f0, min(f0 + TB, Fh), tok)))

            def fin():
                y = _dot(jnp.concatenate(us, axis=1), _bf(wout_ref[...]))
                gate.append(y * (1.0 / (1.0 + jnp.exp(-y))))

            s0, mem = pair_step(it * 2, mem_ref[...], 0, lambda: None, lambda: rest(FU), [])
            s1, mem = pair_step(it * 2 + 1, mem, 1, lambda: rest(FU + TB), lambda: rest(FU + 2 * TB), [fin])
            mem_ref[...] = mem
            o_ref[r, :] = (x_ref[r, :].astype(F32) + jnp.concatenate([s0, s1], axis=0) * gate[0]).astype(BF16)
            pltpu.make_async_copy(o_ref.at[r, :], o_hbm.at[r, :], osem).start()

        loop(NB, step)
        pltpu.make_async_copy(o_ref, o_hbm, osem).wait()

    any_spec = pl.BlockSpec(memory_space=pl.ANY)
    out = pl.pallas_call(
        kern,
        out_shape=jax.ShapeDtypeStruct((S, D), BF16),
        in_specs=[any_spec] * 10,
        out_specs=any_spec,
        scratch_shapes=[
            pltpu.VMEM((S, D), BF16),
            pltpu.VMEM((F // 2, D), U32),
            pltpu.VMEM((3 * H, D2, Dh), U32),
            pltpu.VMEM((H * Dh // 2, D), U32),
            pltpu.VMEM((HF, D), U32),
            pltpu.VMEM((S // 2, S), U32),
            pltpu.VMEM((S, D), BF16),
            pltpu.VMEM((S // 2, D + 128), U32),
            pltpu.VMEM((NB * HF, 2 * TB), U32),
            pltpu.VMEM((NB, 8, TB), F32),
            pltpu.VMEM((M, D), F32),
            pltpu.VMEM((NB * FU // 2, 2 * TB), U32),
            pltpu.VMEM((NB, Fh, TB), F32),
            pltpu.VMEM((FS * HB, D + 128), U32),
            pltpu.VMEM((GB, HB, S), U32),
            pltpu.VMEM((2, SEG, D), U32),
            pltpu.VMEM((M, D), BF16),
            pltpu.VMEM((NB, TB), BF16),
            pltpu.VMEM((NP * L, 3 * Dh), U32),
            pltpu.SemaphoreType.DMA((FI + 2,)),
            pltpu.SemaphoreType.DMA((NU,)),
            pltpu.SemaphoreType.DMA((NU,)),
            pltpu.SemaphoreType.DMA((7,)),
            pltpu.SemaphoreType.DMA,
        ],
        compiler_params=pltpu.CompilerParams(vmem_limit_bytes=120 * 1024 * 1024),
    )(x2, mem0, wq, wk, wv, wo, winT, B_w_sp, b2, B_w_out)
    return out.reshape(1, S, D)


def pallas_recurrent_scan__memory_aug_recurrent_mem_tr__mixer_gmlp__prompt_kernel(A_x, A_mem0, A_Wq, A_Wk, A_Wv, A_Wo, A_seg_len, B_x, B_w_in, B_w_sp, B_b_sp, B_w_out):
    del B_x
    seg = A_seg_len if isinstance(A_seg_len, int) else 32
    return _run(A_x, A_mem0, A_Wq, A_Wk, A_Wv, A_Wo, B_w_in, B_w_sp, B_b_sp, B_w_out, SEG=seg)
```

```python
import functools
import math

import jax
import jax.numpy as jnp
from jax import lax
import jax.experimental.pallas as pl
import jax.experimental.pallas.tpu as pltpu

F32 = jnp.float32
BF16 = jnp.bfloat16
U32 = jnp.uint32
NT = (((1,), (1,)), ((), ()))
EPS = 1e-5


def _gelu(x):
    c = math.sqrt(2.0 / math.pi)
    h = 0.5 * x
    return h + h * jnp.tanh(x * (c + (c * 0.044715) * (x * x)))


def _dot(a, b):
    return jnp.dot(a, b, preferred_element_type=F32)


def _dot_nt(a, b):
    return lax.dot_general(a, b, NT, preferred_element_type=F32)


def _bf(u32_val):
    return pltpu.bitcast(u32_val, BF16)


def _u32(bf_val):
    return pltpu.bitcast(bf_val, U32)


def _token(t):
    b = pltpu.bitcast(t[0:8, 0:128], U32)
    return (b >> 16) >> 16


def _after(x, tok):
    if tok is None:
        return x
    r, c = x.shape
    z = jnp.concatenate([tok] * (r // 8), axis=0)
    z = jnp.concatenate([z] * (c // 128), axis=1)
    return pltpu.bitcast(pltpu.bitcast(x, U32) | z, x.dtype)


def _rows(start, size, align):
    return pl.ds(pl.multiple_of(start, align), size)


@functools.partial(jax.jit, static_argnames=("SEG",))
def _run(A_x, A_mem0, A_Wq, A_Wk, A_Wv, A_Wo, B_w_in, B_w_sp, B_b_sp, B_w_out, *, SEG):
    _, S, D = A_x.shape
    H, Dh = A_Wq.shape[1], A_Wq.shape[2]
    M = A_mem0.shape[1]
    F = B_w_in.shape[1]
    assert (S, D, H, Dh, M, SEG, F) == (2048, 640, 32, 128, 8, 32, 1728) and A_x.shape[0] == 1
    L = SEG + M
    Fh = F // 2
    HF = Fh // 2
    scale = Dh ** -0.5
    NP = H // 2
    D2 = D // 2
    TB = 4 * SEG
    HB = TB // 2
    NB = S // TB
    RC = 144
    NRC = Fh // RC
    PK = 4
    C0 = 2
    FS = 6
    FI = (NB - PK) // FS
    Z1B = 8
    FU = 512
    GB = 4
    NU = NB // GB
    PG = NP // NU

    x2 = A_x.reshape(S, D)
    mem0 = A_mem0.reshape(M, D)
    wq = A_Wq.reshape(D2, 2 * H, Dh)
    wk = A_Wk.reshape(D2, 2 * H, Dh)
    wv = A_Wv.reshape(D2, 2 * H, Dh)
    wo = A_Wo.reshape(H * Dh, D)
    winT = B_w_in.T
    b2 = B_b_sp.reshape(NB, TB)

    def kern(x_hbm, mem0_hbm, wq_hbm, wk_hbm, wv_hbm, wo_hbm, winT_hbm, wsp_hbm, b_hbm, wout_hbm,
             o_hbm,
             x_ref, winT_ref, w_ref, wo_ref, wout_ref, wsp_ref, o_ref,
             xn_ref, z_ref, brow_ref, mem_ref, u_ref, tmp_ref, nxt_ref, lst_ref, xst_ref,
             mem0_ref, b_ref, xsem, wsem, ssem, sem, osem, *st_refs):
        w_hbm = [w.bitcast(U32) for w in (wq_hbm, wk_hbm, wv_hbm)]
        wsp32 = wsp_hbm.bitcast(U32)
        winT32 = winT_hbm.bitcast(U32)

        XB = [0, PK * TB, (PK + 1) * TB] + [min((PK + 1 + (c + 1) * FS) * TB, S) for c in range(FI)]

        def cp_x(c):
            return pltpu.make_async_copy(x_hbm.at[XB[c]:XB[c + 1], :], x_ref.at[XB[c]:XB[c + 1], :], xsem.at[c])

        def cp_ws(k):
            r2 = pl.ds(k * (GB * HB), GB * HB)
            return pltpu.make_async_copy(wsp32.at[r2], wsp_ref.at[r2], ssem.at[k])

        def start_group(k):
            cp_ws(k).start()
            for p in range(k * PG, (k + 1) * PG):
                for j in range(3):
                    for par in range(2):
                        pltpu.make_async_copy(w_hbm[j].at[:, par * NP + p, :],
                                              w_ref.at[6 * p + 2 * j + par], wsem.at[k]).start()

        def wait_group(k):
            cp_ws(k).wait()
            grp = w_ref.at[pl.ds(k * (6 * PG), 6 * PG)]
            pltpu.make_async_copy(grp, grp, wsem.at[k]).wait()

        WA = HF + C0 * RC // 2
        cp_w2a = pltpu.make_async_copy(winT32.at[HF:WA], winT_ref.at[HF:WA], sem.at[0])
        cp_w2b = pltpu.make_async_copy(winT32.at[WA:], winT_ref.at[WA:], sem.at[6])
        cp_w1 = pltpu.make_async_copy(winT32.at[:HF], winT_ref.at[:HF], sem.at[1])
        cp_wo = pltpu.make_async_copy(wo_hbm.bitcast(U32), wo_ref, sem.at[2])
        cp_wout = pltpu.make_async_copy(wout_hbm.bitcast(U32), wout_ref, sem.at[3])
        cp_m = pltpu.make_async_copy(mem0_hbm, mem0_ref, sem.at[4])
        cp_b = pltpu.make_async_copy(b_hbm, b_ref, sem.at[5])

        cp_x(0).start()
        cp_w2a.start()
        cp_w2b.start()
        for c in range(1, FI + 2):
            cp_x(c).start()
        cp_b.start()
        cp_m.start()
        cp_w1.start()
        start_group(0)
        start_group(1)

        def loop(n, fn):
            def body(c, carry):
                fn(c)
                return carry
            lax.fori_loop(0, n, body, 0)

        def norm_slab(hrow, srow, tok=None):
            x = _after(x_ref[_rows(hrow * 2, 16, 16), :].astype(F32), tok)
            d = x - jnp.sum(x, axis=-1, keepdims=True) * (1.0 / D)
            xn = d * lax.rsqrt(jnp.sum(d * d, axis=-1, keepdims=True) * (1.0 / D) + EPS)
            xu = _u32(xn.astype(BF16))
            xn_ref[_rows(hrow, 8, 8), 0:D] = xu
            nxt_ref[srow:srow + 8, 0:D] = xu

        def z2_chunk(xn, j, n):
            t = _dot_nt(_bf(winT_ref[HF + n * RC // 2:HF + (n + 1) * RC // 2, :]), xn)
            tmp_ref[j, n * RC:(n + 1) * RC, :] = _gelu(t)
            return t

        def front2(c):
            for k in range(FI):
                @pl.when(c == k)
                def _():
                    cp_x(k + 2).wait()
            rel = [-2, -2, -1, -1, 0, 0, 1, 2]
            prev = {}
            for s in range(FS):
                j = PK + c * FS + s
                nrow = (j + 1) * HB
                if s == FS - 1:
                    nrow = jnp.minimum(nrow, (NB - 1) * HB)
                xn = _bf(nxt_ref[s * HB:(s + 1) * HB, 0:D])
                srow = ((s + 1) % FS) * HB
                for i in range(8):
                    if rel[i] < 0:
                        norm_slab(nrow + i * 8, srow + i * 8, prev.get(NRC + rel[i]))
                cur = {}
                for n in range(NRC):
                    cur[n] = _token(z2_chunk(xn, j, n))
                    for i in range(8):
                        if rel[i] == n:
                            norm_slab(nrow + i * 8, srow + i * 8, cur[n])
                prev = cur

        def ln_block(j, tok):
            G = 48
            rep = lambda v: jnp.concatenate([v] * (G // 8), axis=0)
            acc = pltpu.bitcast(tok, F32)
            for q in range(0, Fh, 8):
                acc = acc + tmp_ref[j, q:q + 8, :]
            mean = jnp.broadcast_to(jnp.sum(acc, axis=0, keepdims=True) * (1.0 / Fh), (8, TB))
            acc = None
            for q in range(0, Fh, G):
                m = mean if acc is None else _after(mean, _token(acc))
                d = tmp_ref[j, q:q + G, :] - rep(m)
                part = jnp.sum((d * d).reshape(G // 8, 8, TB), axis=0)
                acc = part if acc is None else acc + part
            rstd = lax.rsqrt(jnp.sum(acc, axis=0, keepdims=True) * (1.0 / Fh) + EPS)
            tok = _token(jnp.broadcast_to(rstd, (8, TB)))
            for q in range(0, Fh, G):
                o = (tmp_ref[j, q:q + G, :] - rep(_after(mean, tok))) * rstd
                z_ref[_rows(j * HF + q // 2, G // 2, 8), TB:2 * TB] = _u32(o.astype(BF16))
                tok = _token(o)

        def front1(c):
            tok = None
            for s in range(Z1B):
                j = c * Z1B + s
                xu = xn_ref[_rows(j * HB, HB, HB), 0:D]
                if tok is None:
                    tok = _token(xu)
                    ln_block(j, tok)
                xn = _bf(_after(xu, tok))
                for n in range(NRC):
                    t = _dot_nt(_bf(winT_ref[n * RC // 2:(n + 1) * RC // 2, :]), xn)
                    z_ref[_rows(j * HF + n * RC // 2, RC // 2, 8), 0:TB] = _u32(_gelu(t).astype(BF16))
                    if n == 2:
                        tok = _token(t)
                    if n == 3 and s + 1 < Z1B:
                        ln_block(j + 1, _token(t))

        def stage_ws(j, slot):
            lst_ref[slot] = wsp_ref[_rows(j * HB, HB, HB), :]

        def ut_part(j, slot, f0, f1):
            zs = [z_ref[k * HF + f0 // 2:k * HF + f1 // 2, TB:2 * TB] for k in range(NB)]
            gt = _dot_nt(_bf(jnp.concatenate(zs, axis=1)), _bf(lst_ref[slot]))
            z1t = _bf(z_ref[_rows(j * HF + f0 // 2, (f1 - f0) // 2, 8), 0:TB]).astype(F32)
            bt = jnp.concatenate([brow_ref[j]] * ((f1 - f0) // 8), axis=0)
            return z1t * gt + z1t * bt

        def untranspose(ut):
            n = ut.shape[0]
            if n < TB:
                ut = jnp.concatenate([ut, jnp.zeros((TB - n, TB), F32)], axis=0)
            return ut.T[:, :n].astype(BF16)

        def relayout(k, tok):
            G = 16
            for i in range(3 * PG):
                sa = k * (6 * PG) + 2 * i
                for q in range(0, D2, G):
                    lo = jnp.concatenate([tok | U32(0xFFFF)] * (G // 8), axis=0)
                    hi = jnp.concatenate([tok | U32(0xFFFF0000)] * (G // 8), axis=0)
                    a = w_ref[sa, q:q + G, :]
                    b = w_ref[sa + 1, q:q + G, :]
                    h0 = (a & lo) | (b << 16)
                    w_ref[sa, q:q + G, :] = h0
                    w_ref[sa + 1, q:q + G, :] = (a >> 16) | (b & hi)
                    tok = _token(h0)

        def upfront(c):
            wait_group(c)
            for s in range(GB):
                j = c * GB + s
                stage_ws(j, s)
                for f0 in range(0, FU, TB):
                    ut = ut_part(j, s, f0, f0 + TB)
                    u_ref[_rows(j * (FU // 2) + f0 // 2, HB, 8), 0:TB] = _u32(ut.astype(BF16))
                    if s == 0 and f0 == 0:
                        relayout(c, _token(ut))

        cp_x(0).wait()
        for i in range(16):
            norm_slab(i * 8, HB + i * 8)
        cp_w2a.wait()
        for i in range(16, 8 * PK):
            norm_slab(i * 8, HB + i * 8)
        for j in range(PK):
            for n in range(C0):
                z2_chunk(_bf(nxt_ref[(j + 1) * HB:(j + 2) * HB, 0:D]), j, n)
        cp_w2b.wait()
        cp_x(1).wait()
        i = 0
        for j in range(PK):
            for n in range(C0, NRC):
                t = z2_chunk(_bf(nxt_ref[(j + 1) * HB:(j + 2) * HB, 0:D]), j, n)
                if i < 8:
                    norm_slab(PK * HB + i * 8, i * 8, _token(t))
                    i += 1

        loop(FI, front2)
        start_group(2)
        cp_b.wait()
        cp_m.wait()
        bf32 = b_ref[...].astype(F32)
        for i in range(NB):
            brow_ref[i] = jnp.broadcast_to(bf32[i:i + 1, :], (8, TB))
        mem_ref[...] = mem0_ref[...].astype(F32)
        cp_w1.wait()
        loop(NB // Z1B, front1)
        start_group(3)
        cp_wout.start()
        cp_wo.start()
        loop(NU, upfront)
        cp_wout.wait()
        cp_wo.wait()

        ri = lax.broadcasted_iota(jnp.int32, (2 * L, 2 * L), 0)
        ci = lax.broadcasted_iota(jnp.int32, (2 * L, 2 * L), 1)
        rh = ri >= L
        ch = ci >= L
        rr = jnp.where(rh, ri - L, ri)
        cc = jnp.where(ch, ci - L, ci)
        same = rh == ch
        valid = same & ((rr >= SEG) | (cc >= SEG) | (rr >= cc))
        fill = jnp.where(same, -1e9 / scale, -jnp.inf).astype(F32)
        mask = {skip: tuple(jnp.concatenate([a[skip:L], a[L + skip:]], axis=0) for a in (valid, fill))
                for skip in (0, M, 2 * M)}
        sub = lax.broadcasted_iota(jnp.int32, (M, Dh), 0)
        c2 = scale * math.log2(math.e)
        neg = -1e9 * math.log2(math.e)
        add = lambda xs: functools.reduce(lambda a, b: a + b, xs)
        both = lambda toks: functools.reduce(lambda a, b: a | b, toks)

        def recip(den):
            inv = pl.reciprocal(den, approx=True)
            return inv * (2.0 - den * inv)

        def head_rows(q, kd, vd, kf, vf):
            q = q * c2
            rot = lambda a, r: pltpu.roll(a, r, 0) if r else a
            red = lambda a: jnp.broadcast_to(jnp.sum(a, axis=-1, keepdims=True), (M, Dh))
            sc = [None] * M
            sc[0] = red(q * kd)
            sc[M // 2] = jnp.where(sub >= M // 2, red(q * rot(kd, M // 2)), neg)
            for r in range(1, M // 2):
                t = red(jnp.where(sub >= r, q * rot(kd, r), rot(q, r) * kd))
                sc[r] = jnp.where(sub >= r, t, neg)
                sc[M - r] = jnp.where(sub >= M - r, rot(t, M - r), neg)
            sc += [red(q * rot(k, r)) for k in kf for r in range(M)]
            mx = functools.reduce(jnp.maximum, sc)
            e = [jnp.exp2(t - mx) for t in sc]
            o = add([e[b * M + r] * rot(v, r) for b, v in enumerate([vd] + vf) for r in range(M)])
            return o * recip(add(e))

        wgate = {}

        def wpair(p):
            ws = []
            for i in range(6):
                w = w_ref[6 * p + i]
                if 6 * p + i in wgate:
                    w = jnp.concatenate([w[:D2 - 8], w[D2 - 8:] | wgate.pop(6 * p + i)], axis=0)
                ws.append(w)
            return _bf(jnp.concatenate(ws, axis=1))

        def segment(first, proj, wo_lhs, extra, wo_groups, zero, hold):
            pm, ov, oc, acc = {}, {}, {}, []
            skip = lambda p: 0 if (not first or p >= NP - 2) else (M if p % 2 else 2 * M)

            def qkv(p, j):
                n = L - skip(p) if j == 0 else L
                return _bf(st_refs[p][0:n, j * Dh:(j + 1) * Dh])

            def project(p):
                t = proj(p)
                for j in range(3):
                    lo = skip(p) if j == 0 else 0
                    two = jnp.concatenate([t[lo:, 2 * j * Dh:(2 * j + 1) * Dh],
                                           t[lo:, (2 * j + 1) * Dh:(2 * j + 2) * Dh]], axis=0)
                    st_refs[p][_rows(zero, L - lo, 8), j * Dh:(j + 1) * Dh] = _u32(two.astype(BF16))
                blk = lambda i, b: t[b * M:(b + 1) * M, i * Dh:(i + 1) * Dh]
                seen = lambda b: list(range(b)) + [SEG // M]
                ov[p] = [jnp.concatenate(
                    [head_rows(blk(e, b), blk(2 + e, b), blk(4 + e, b), [blk(2 + e, f) for f in seen(b)],
                               [blk(4 + e, f) for f in seen(b)]) for e in range(2)], axis=1)
                    for b in range(skip(p) // M)]
                toks = [_token(o[:, e * Dh:]) for o in ov[p] for e in range(2)]
                for tok, off in zip(toks, (1, 5) if len(toks) == 2 else (2, 4, 6, 9)):
                    wgate[6 * (p + 2) + off] = tok

            def score(p):
                valid, fill = mask[skip(p)]
                sc = jnp.where(valid, _dot_nt(qkv(p, 0), qkv(p, 1)), fill)
                mx = jnp.max(sc, axis=-1, keepdims=True)
                e = jnp.exp2((sc - mx) * c2)
                e = e * recip(jnp.sum(e, axis=-1, keepdims=True))
                if first:
                    if p == NP - 3:
                        e = jnp.concatenate(
                            [pltpu.bitcast(pltpu.bitcast(e[:8], U32) | hold[:, :2 * L], F32), e[8:]], axis=0)
                    pm[p] = e.astype(BF16)
                else:
                    st_refs[NP + p][_rows(zero, L, 8), 0:2 * L] = _u32(e.astype(BF16))

            def pv(p):
                n = L - skip(p)
                o2 = _dot(pm[p] if first else _bf(st_refs[NP + p][:, 0:2 * L]), qkv(p, 2))
                oc[p] = jnp.concatenate(ov[p] + [jnp.concatenate([o2[:n], o2[n:]], axis=1)], axis=0)

            def wo(ps):
                lhs = jnp.concatenate([wo_lhs(p, oc[p]) for p in ps], axis=1).astype(BF16)
                t = _dot(lhs, _bf(wo_ref[ps[0] * Dh:(ps[-1] + 1) * Dh, :]))
                acc[:] = [t + acc[0] if acc else t]

            fillers = extra + [functools.partial(wo, range(*g)) for g in wo_groups]
            if first:
                for i in range(NP + 3):
                    if i < NP:
                        project(i)
                    else:
                        fillers.pop(0)()
                    if 1 <= i <= NP:
                        score(i - 1)
                    if i >= 3:
                        pv(i - 3)
            else:
                for g in range(NP // 4 + 2):
                    last = g >= NP // 4
                    for k in range(1 if last else 4):
                        if last:
                            fillers.pop(0)()
                        else:
                            project(4 * g + k)
                        if last or k == 1:
                            for p in range(4 * g - 8, 4 * g - 4) if g >= 2 else ():
                                pv(p)
                            for p in range(4 * g - 4, 4 * g) if 1 <= g <= NP // 4 else ():
                                score(p)
            for f in fillers:
                f()
            return acc[0], oc

        def pair_step(ip, mem_a, slot, fill_b, extra, wo_groups, zero, hold):
            xst_ref[slot] = xn_ref[_rows(ip * SEG, SEG, SEG), 0:D]
            xs = _bf(xst_ref[slot])
            xb = xs[SEG:].astype(F32)
            ha = jnp.concatenate([xs[:SEG], jnp.concatenate([xb[:M], mem_a], axis=0).astype(BF16)], axis=0)
            early = {}

            def proj_a(p):
                t = _dot(ha, wpair(p))
                early[p] = t[SEG:SEG + M]
                return jnp.concatenate([t[:SEG], t[SEG + M:]], axis=0)

            acc_a, oca = segment(True, proj_a, lambda p, o: o[M:], [],
                                 ((0, 2 + 2 * slot), (2 + 2 * slot, 6), (6, 10), (10, 14), (14, 16)), zero, hold)
            mem_b = acc_a[SEG - M:].astype(BF16).astype(F32)
            fill_b()
            hb = jnp.concatenate([xb[M:], mem_b], axis=0).astype(BF16)
            acc_b, _ = segment(False, lambda p: jnp.concatenate([early[p], _dot(hb, wpair(p))], axis=0),
                               lambda p, o: jnp.concatenate([oca[p][:M], o], axis=0), extra, wo_groups, zero, None)
            sa = jnp.concatenate([acc_b[:M], acc_a[:SEG - M], acc_b[M:SEG + M]], axis=0)
            return sa, acc_b[SEG + M:].astype(BF16).astype(F32)

        def step(it):
            r = _rows(it * TB, TB, TB)
            zero = (it >> 10) * 8
            stage_ws(it, 0)
            us = [untranspose(_bf(u_ref[_rows(it * (FU // 2) + f0 // 2, HB, 8), 0:TB]).astype(F32))
                  for f0 in range(0, FU, TB)]
            gate = []
            done = lambda parts: both([_token(_u32(u)[HB - 8:]) for u in parts])

            def rest(f0):
                us.append(untranspose(ut_part(it, 0, f0, min(f0 + TB, Fh))))

            def fin():
                y = _dot(jnp.concatenate(us, axis=1), _bf(wout_ref[...]))
                gate.append(y * (1.0 / (1.0 + jnp.exp(-y))))

            s0, mem = pair_step(it * 2, mem_ref[...], 0, lambda: rest(FU), [],
                                ((0, 2), (2, 8), (8, 12), (12, 16)), zero, done(us))
            rest(FU + TB)
            s1, mem = pair_step(it * 2 + 1, mem, 1, lambda: rest(FU + 2 * TB), [fin],
                                ((0, 6), (6, 12), (12, 16)), zero, done(us[FU // TB:]))
            mem_ref[...] = mem
            o_ref[r, :] = (x_ref[r, :].astype(F32) + jnp.concatenate([s0, s1], axis=0) * gate[0]).astype(BF16)
            pltpu.make_async_copy(o_ref.at[r, :], o_hbm.at[r, :], osem).start()

        loop(NB, step)
        pltpu.make_async_copy(o_ref, o_hbm, osem).wait()

    any_spec = pl.BlockSpec(memory_space=pl.ANY)
    out = pl.pallas_call(
        kern,
        out_shape=jax.ShapeDtypeStruct((S, D), BF16),
        in_specs=[any_spec] * 10,
        out_specs=any_spec,
        scratch_shapes=[
            pltpu.VMEM((S, D), BF16),
            pltpu.VMEM((F // 2, D), U32),
            pltpu.VMEM((3 * H, D2, Dh), U32),
            pltpu.VMEM((H * Dh // 2, D), U32),
            pltpu.VMEM((HF, D), U32),
            pltpu.VMEM((S // 2, S), U32),
            pltpu.VMEM((S, D), BF16),
            pltpu.VMEM((S // 2, D + 128), U32),
            pltpu.VMEM((NB * HF, 2 * TB), U32),
            pltpu.VMEM((NB, 8, TB), F32),
            pltpu.VMEM((M, D), F32),
            pltpu.VMEM((NB * FU // 2, 2 * TB), U32),
            pltpu.VMEM((NB, Fh, TB), F32),
            pltpu.VMEM((FS * HB, D + 128), U32),
            pltpu.VMEM((GB, HB, S), U32),
            pltpu.VMEM((2, SEG, D), U32),
            pltpu.VMEM((M, D), BF16),
            pltpu.VMEM((NB, TB), BF16),
            pltpu.SemaphoreType.DMA((FI + 2,)),
            pltpu.SemaphoreType.DMA((NU,)),
            pltpu.SemaphoreType.DMA((NU,)),
            pltpu.SemaphoreType.DMA((7,)),
            pltpu.SemaphoreType.DMA,
        ] + [pltpu.VMEM((L, 3 * Dh), U32)] * NP
          + [pltpu.VMEM((L, 128), U32)] * NP,
        compiler_params=pltpu.CompilerParams(vmem_limit_bytes=120 * 1024 * 1024),
    )(x2, mem0, wq, wk, wv, wo, winT, B_w_sp, b2, B_w_out)
    return out.reshape(1, S, D)


def pallas_recurrent_scan__memory_aug_recurrent_mem_tr__mixer_gmlp__prompt_kernel(A_x, A_mem0, A_Wq, A_Wk, A_Wv, A_Wo, A_seg_len, B_x, B_w_in, B_w_sp, B_b_sp, B_w_out):
    del B_x
    seg = A_seg_len if isinstance(A_seg_len, int) else 32
    return _run(A_x, A_mem0, A_Wq, A_Wk, A_Wv, A_Wo, B_w_in, B_w_sp, B_b_sp, B_w_out, SEG=seg)
```

```python
import functools
import math

import jax
import jax.numpy as jnp
from jax import lax
import jax.experimental.pallas as pl
import jax.experimental.pallas.tpu as pltpu

F32 = jnp.float32
BF16 = jnp.bfloat16
U32 = jnp.uint32
NT = (((1,), (1,)), ((), ()))
EPS = 1e-5


def _gelu(x):
    c = math.sqrt(2.0 / math.pi)
    h = 0.5 * x
    return h + h * jnp.tanh(x * (c + (c * 0.044715) * (x * x)))


def _silu(y):
    h = 0.5 * y
    return h + h * jnp.tanh(h)


def _dot(a, b):
    return jnp.dot(a, b, preferred_element_type=F32)


def _dot_nt(a, b):
    return lax.dot_general(a, b, NT, preferred_element_type=F32)


def _bf(u32_val):
    return pltpu.bitcast(u32_val, BF16)


def _u32(bf_val):
    return pltpu.bitcast(bf_val, U32)


def _token(t):
    b = pltpu.bitcast(t[0:8, 0:128], U32)
    return (b >> 16) >> 16


def _after(x, tok):
    if tok is None:
        return x
    r, c = x.shape
    z = jnp.concatenate([tok] * (r // 8), axis=0)
    z = jnp.concatenate([z] * (c // 128), axis=1)
    return pltpu.bitcast(pltpu.bitcast(x, U32) | z, x.dtype)


def _rows(start, size, align):
    return pl.ds(pl.multiple_of(start, align), size)


@functools.partial(jax.jit, static_argnames=("SEG",))
def _run(A_x, A_mem0, A_Wq, A_Wk, A_Wv, A_Wo, B_w_in, B_w_sp, B_b_sp, B_w_out, *, SEG):
    _, S, D = A_x.shape
    H, Dh = A_Wq.shape[1], A_Wq.shape[2]
    M = A_mem0.shape[1]
    F = B_w_in.shape[1]
    assert (S, D, H, Dh, M, SEG, F) == (2048, 640, 32, 128, 8, 32, 1728) and A_x.shape[0] == 1
    L = SEG + M
    Fh = F // 2
    HF = Fh // 2
    scale = Dh ** -0.5
    NP = H // 2
    D2 = D // 2
    TB = 4 * SEG
    HB = TB // 2
    NB = S // TB
    RC = 144
    NRC = Fh // RC
    PK = 4
    C0 = 2
    FS = 6
    FI = (NB - PK) // FS
    Z1B = 8
    FU = 512
    GB = 4
    NU = NB // GB
    PG = NP // NU

    x2 = A_x.reshape(S, D)
    mem0 = A_mem0.reshape(M, D)
    wq = A_Wq.reshape(D2, 2 * H, Dh)
    wk = A_Wk.reshape(D2, 2 * H, Dh)
    wv = A_Wv.reshape(D2, 2 * H, Dh)
    wo = A_Wo.reshape(H * Dh, D)
    winT = B_w_in.T
    b2 = B_b_sp.reshape(NB, TB)

    def kern(x_hbm, mem0_hbm, wq_hbm, wk_hbm, wv_hbm, wo_hbm, winT_hbm, wsp_hbm, b_hbm, wout_hbm,
             o_hbm,
             x_ref, winT_ref, w_ref, wo_ref, wout_ref, wsp_ref, o_ref,
             xn_ref, z_ref, brow_ref, mem_ref, u_ref, tmp_ref, nxt_ref, lst_ref, ear_ref,
             mem0_ref, b_ref, xsem, wsem, ssem, sem, osem, *st_refs):
        w_hbm = [w.bitcast(U32) for w in (wq_hbm, wk_hbm, wv_hbm)]
        wsp32 = wsp_hbm.bitcast(U32)
        winT32 = winT_hbm.bitcast(U32)

        XB = [0, PK * TB, (PK + 1) * TB] + [min((PK + 1 + (c + 1) * FS) * TB, S) for c in range(FI)]

        def cp_x(c):
            return pltpu.make_async_copy(x_hbm.at[XB[c]:XB[c + 1], :], x_ref.at[XB[c]:XB[c + 1], :], xsem.at[c])

        def cp_ws(k):
            r2 = pl.ds(k * (GB * HB), GB * HB)
            return pltpu.make_async_copy(wsp32.at[r2], wsp_ref.at[r2], ssem.at[k])

        def start_group(k):
            cp_ws(k).start()
            for p in range(k * PG, (k + 1) * PG):
                for j in range(3):
                    for par in range(2):
                        pltpu.make_async_copy(w_hbm[j].at[:, par * NP + p, :],
                                              w_ref.at[6 * p + 2 * j + par], wsem.at[k]).start()

        def wait_group(k):
            cp_ws(k).wait()
            grp = w_ref.at[pl.ds(k * (6 * PG), 6 * PG)]
            pltpu.make_async_copy(grp, grp, wsem.at[k]).wait()

        WA = HF + C0 * RC // 2
        cp_w2a = pltpu.make_async_copy(winT32.at[HF:WA], winT_ref.at[HF:WA], sem.at[0])
        cp_w2b = pltpu.make_async_copy(winT32.at[WA:], winT_ref.at[WA:], sem.at[6])
        cp_w1 = pltpu.make_async_copy(winT32.at[:HF], winT_ref.at[:HF], sem.at[1])
        cp_wo = pltpu.make_async_copy(wo_hbm.bitcast(U32), wo_ref, sem.at[2])
        cp_wout = pltpu.make_async_copy(wout_hbm.bitcast(U32), wout_ref, sem.at[3])
        cp_m = pltpu.make_async_copy(mem0_hbm, mem0_ref, sem.at[4])
        cp_b = pltpu.make_async_copy(b_hbm, b_ref, sem.at[5])

        cp_x(0).start()
        cp_w2a.start()
        cp_w2b.start()
        for c in range(1, FI + 2):
            cp_x(c).start()
        cp_b.start()
        cp_m.start()
        cp_w1.start()
        start_group(0)
        start_group(1)

        def loop(n, fn):
            def body(c, carry):
                fn(c)
                return carry
            lax.fori_loop(0, n, body, 0)

        def norm_slab(hrow, srow, tok=None):
            x = _after(x_ref[_rows(hrow * 2, 16, 16), :].astype(F32), tok)
            d = x - jnp.sum(x, axis=-1, keepdims=True) * (1.0 / D)
            xn = d * lax.rsqrt(jnp.sum(d * d, axis=-1, keepdims=True) * (1.0 / D) + EPS)
            xu = _u32(xn.astype(BF16))
            xn_ref[_rows(hrow, 8, 8), 0:D] = xu
            nxt_ref[srow:srow + 8, 0:D] = xu

        def z2_chunk(xn, j, n):
            t = _dot_nt(_bf(winT_ref[HF + n * RC // 2:HF + (n + 1) * RC // 2, :]), xn)
            tmp_ref[j, n * RC:(n + 1) * RC, :] = _gelu(t)
            return t

        def front2(c):
            for k in range(FI):
                @pl.when(c == k)
                def _():
                    cp_x(k + 2).wait()
            rel = [-2, -2, -1, -1, 0, 0, 1, 2]
            prev = {}
            for s in range(FS):
                j = PK + c * FS + s
                nrow = (j + 1) * HB
                if s == FS - 1:
                    nrow = jnp.minimum(nrow, (NB - 1) * HB)
                xn = _bf(nxt_ref[s * HB:(s + 1) * HB, 0:D])
                srow = ((s + 1) % FS) * HB
                for i in range(8):
                    if rel[i] < 0:
                        norm_slab(nrow + i * 8, srow + i * 8, prev.get(NRC + rel[i]))
                cur = {}
                for n in range(NRC):
                    cur[n] = _token(z2_chunk(xn, j, n))
                    for i in range(8):
                        if rel[i] == n:
                            norm_slab(nrow + i * 8, srow + i * 8, cur[n])
                prev = cur

        def ln_block(j, tok):
            G = 48
            rep = lambda v: jnp.concatenate([v] * (G // 8), axis=0)
            acc = pltpu.bitcast(tok, F32)
            for q in range(0, Fh, 8):
                acc = acc + tmp_ref[j, q:q + 8, :]
            mean = jnp.broadcast_to(jnp.sum(acc, axis=0, keepdims=True) * (1.0 / Fh), (8, TB))
            acc = None
            for q in range(0, Fh, G):
                m = mean if acc is None else _after(mean, _token(acc))
                d = tmp_ref[j, q:q + G, :] - rep(m)
                part = jnp.sum((d * d).reshape(G // 8, 8, TB), axis=0)
                acc = part if acc is None else acc + part
            rstd = lax.rsqrt(jnp.sum(acc, axis=0, keepdims=True) * (1.0 / Fh) + EPS)
            tok = _token(jnp.broadcast_to(rstd, (8, TB)))
            for q in range(0, Fh, G):
                o = (tmp_ref[j, q:q + G, :] - rep(_after(mean, tok))) * rstd
                z_ref[_rows(j * HF + q // 2, G // 2, 8), TB:2 * TB] = _u32(o.astype(BF16))
                tok = _token(o)

        def front1(c):
            tok = None
            for s in range(Z1B):
                j = c * Z1B + s
                xu = xn_ref[_rows(j * HB, HB, HB), 0:D]
                if tok is None:
                    tok = _token(xu)
                    ln_block(j, tok)
                xn = _bf(_after(xu, tok))
                for n in range(NRC):
                    t = _dot_nt(_bf(winT_ref[n * RC // 2:(n + 1) * RC // 2, :]), xn)
                    z_ref[_rows(j * HF + n * RC // 2, RC // 2, 8), 0:TB] = _u32(_gelu(t).astype(BF16))
                    if n == 2:
                        tok = _token(t)
                    if n == 3 and s + 1 < Z1B:
                        ln_block(j + 1, _token(t))

        def stage_ws(j, slot):
            lst_ref[slot] = wsp_ref[_rows(j * HB, HB, HB), :]

        def ut_part(j, slot, f0, f1, between=None):
            zs = [z_ref[k * HF + f0 // 2:k * HF + f1 // 2, TB:2 * TB] for k in range(NB)]
            if between is None:
                gt = _dot_nt(_bf(jnp.concatenate(zs, axis=1)), _bf(lst_ref[slot]))
            else:
                gt = None
                for k in range(0, NB, 4):
                    t = _dot_nt(_bf(jnp.concatenate(zs[k:k + 4], axis=1)),
                                _bf(lst_ref[slot, :, k * TB:(k + 4) * TB]))
                    gt = t if gt is None else t + gt
                    between()
            z1t = _bf(z_ref[_rows(j * HF + f0 // 2, (f1 - f0) // 2, 8), 0:TB]).astype(F32)
            bt = jnp.concatenate([brow_ref[j]] * ((f1 - f0) // 8), axis=0)
            return z1t * gt + z1t * bt

        def untranspose(ut):
            n = ut.shape[0]
            if n < TB:
                ut = jnp.concatenate([ut, jnp.zeros((TB - n, TB), F32)], axis=0)
            return ut.T[:, :n].astype(BF16)

        def relayout(k, tok):
            G = 16
            for i in range(3 * PG):
                sa = k * (6 * PG) + 2 * i
                for q in range(0, D2, G):
                    lo = jnp.concatenate([tok | U32(0xFFFF)] * (G // 8), axis=0)
                    hi = jnp.concatenate([tok | U32(0xFFFF0000)] * (G // 8), axis=0)
                    a = w_ref[sa, q:q + G, :]
                    b = w_ref[sa + 1, q:q + G, :]
                    h0 = (a & lo) | (b << 16)
                    w_ref[sa, q:q + G, :] = h0
                    w_ref[sa + 1, q:q + G, :] = (a >> 16) | (b & hi)
                    tok = _token(h0)

        def upfront(c):
            wait_group(c)
            x0 = _bf(xn_ref[0:8, 0:D])
            tiles = [(q, i, kt) for q in range(PG // 2) for i in range(6) for kt in range(D // 128)]
            acc = {}

            def between():
                for q, i, kt in [tiles.pop(0) for _ in range(min(4, len(tiles)))]:
                    w = w_ref[6 * (c * PG + 2 * q + 1) + i, kt * 64:(kt + 1) * 64, :]
                    t = _dot(x0[:, kt * 128:(kt + 1) * 128], _bf(w))
                    acc[0] = t + acc[0] if kt else t
                    if kt == D // 128 - 1:
                        ear_ref[c * (PG // 2) + q, :, i * Dh:(i + 1) * Dh] = acc[0][:M]

            for s in range(GB):
                j = c * GB + s
                stage_ws(j, s)
                for f0 in range(0, FU, TB):
                    ut = ut_part(j, s, f0, f0 + TB, between if s == 2 else None)
                    u_ref[_rows(j * (FU // 2) + f0 // 2, HB, 8), 0:TB] = _u32(ut.astype(BF16))
                    if s == 0 and f0 == 0:
                        relayout(c, _token(ut))
            assert not tiles

        cp_x(0).wait()
        for i in range(16):
            norm_slab(i * 8, HB + i * 8)
        cp_w2a.wait()
        for i in range(16, 8 * PK):
            norm_slab(i * 8, HB + i * 8)
        for j in range(PK):
            for n in range(C0):
                z2_chunk(_bf(nxt_ref[(j + 1) * HB:(j + 2) * HB, 0:D]), j, n)
        cp_w2b.wait()
        cp_x(1).wait()
        i = 0
        for j in range(PK):
            for n in range(C0, NRC):
                t = z2_chunk(_bf(nxt_ref[(j + 1) * HB:(j + 2) * HB, 0:D]), j, n)
                if i < 8:
                    norm_slab(PK * HB + i * 8, i * 8, _token(t))
                    i += 1

        loop(FI, front2)
        start_group(2)
        cp_b.wait()
        cp_m.wait()
        bf32 = b_ref[...].astype(F32)
        for i in range(NB):
            brow_ref[i] = jnp.broadcast_to(bf32[i:i + 1, :], (8, TB))
        mem_ref[...] = mem0_ref[...].astype(F32)
        cp_w1.wait()
        loop(NB // Z1B, front1)
        start_group(3)
        cp_wout.start()
        cp_wo.start()
        loop(NU, upfront)
        cp_wout.wait()
        cp_wo.wait()

        ri = lax.broadcasted_iota(jnp.int32, (2 * SEG, 2 * L), 0)
        ci = lax.broadcasted_iota(jnp.int32, (2 * SEG, 2 * L), 1)
        rh = ri >= SEG
        ch = ci >= L
        rr = jnp.where(rh, ri - SEG, ri) + M
        cc = jnp.where(ch, ci - L, ci)
        same = rh == ch
        valid = same & ((rr >= SEG) | (cc >= SEG) | (rr >= cc))
        fill = jnp.where(same, -1e9 / scale, -jnp.inf).astype(F32)
        sub = lax.broadcasted_iota(jnp.int32, (M, Dh), 0)
        c2 = scale * math.log2(math.e)
        neg = -1e9 * math.log2(math.e)
        add = lambda xs: functools.reduce(lambda a, b: a + b, xs)

        def recip(den):
            inv = pl.reciprocal(den, approx=True)
            return inv * (2.0 - den * inv)

        def head_rows(q, kx, vx, km, vm):
            q = q * c2
            rot = lambda a, r: pltpu.roll(a, r, 0) if r else a
            red = lambda a: jnp.broadcast_to(jnp.sum(a, axis=-1, keepdims=True), (M, Dh))
            sc = [None] * M
            for r in range(1, M // 2):
                t = red(jnp.where(sub >= r, q * rot(kx, r), rot(q, r) * kx))
                sc[r] = jnp.where(sub >= r, t, neg)
                sc[M - r] = jnp.where(sub >= M - r, rot(t, M - r), neg)
            sc[0] = red(q * kx)
            sc[M // 2] = jnp.where(sub >= M // 2, red(q * rot(kx, M // 2)), neg)
            sc += [red(q * rot(km, r)) for r in range(M)]
            mx = functools.reduce(jnp.maximum, sc)
            e = [jnp.exp2(t - mx) for t in sc]
            o = add([e[b * M + r] * rot(v, r) for b, v in enumerate((vx, vm)) for r in range(M)])
            return o * recip(add(e))

        wgate = {}

        def segment(sidx, hs, hx, early_in, prev_rows, extra, wo_groups, zero, hold=None):
            pm, ov, oc, acc, early = {}, {}, {}, [], {}
            hl = jnp.concatenate([hs, hx], axis=0)
            NG = NP // 2
            nxt, ogate = [0], {}
            odead = [(0, 3), (2, 0), (2, 1), (2, 2), (2, 3), (2, 4), (8, 0), (8, 2)]

            def qkv(p, j):
                return _bf(st_refs[p][0:(L if j else SEG), j * Dh:(j + 1) * Dh])

            def project(g):
                cols = {2 * g: [], 2 * g + 1: []}
                for i in range(6):
                    for p in cols:
                        w = w_ref[6 * p + i]
                        pos = 12 * g + 2 * i + p % 2
                        if pos in wgate:
                            w = jnp.concatenate([w[:D2 - 8], w[D2 - 8:] | wgate.pop(pos)], axis=0)
                        cols[p].append(_dot(hs if (p + sidx) % 2 else hl, _bf(w)))
                    if i == 2:
                        attend(g)
                for p in cols:
                    t = jnp.concatenate(cols[p], axis=1)
                    if (p + sidx) % 2:
                        t = jnp.concatenate([early_in(p), t], axis=0)
                    else:
                        early[p] = t[SEG + M:]
                        t = jnp.concatenate([t[SEG:SEG + M], t[:SEG]], axis=0)
                    for j in range(3):
                        lo = 0 if j else M
                        two = jnp.concatenate([t[lo:, 2 * j * Dh:(2 * j + 1) * Dh],
                                               t[lo:, (2 * j + 1) * Dh:(2 * j + 2) * Dh]], axis=0)
                        st_refs[p][_rows(zero, L - lo, 8), j * Dh:(j + 1) * Dh] = _u32(two.astype(BF16))
                    cx = lambda i: t[:M, i * Dh:(i + 1) * Dh]
                    cm = lambda i: t[SEG:, i * Dh:(i + 1) * Dh]
                    ov[p] = jnp.concatenate(
                        [head_rows(cx(e), cx(2 + e), cx(4 + e), cm(2 + e), cm(4 + e)) for e in range(2)], axis=1)
                    for e in range(2):
                        nxt[0] = max(12 * (g + 1) + 10, nxt[0] + 3)
                        tok = _token(ov[p][:, e * Dh:])
                        if nxt[0] < 12 * NG or sidx % 2 == 0:
                            wgate[nxt[0] % (12 * NG)] = tok
                        else:
                            ogate[odead.pop(0)] = tok

            def score(p):
                sc = jnp.where(valid, _dot_nt(qkv(p, 0), qkv(p, 1)), fill)
                mx = jnp.max(sc, axis=-1, keepdims=True)
                e = jnp.exp2((sc - mx) * c2)
                e = e * recip(jnp.sum(e, axis=-1, keepdims=True))
                if hold is not None and p == 11:
                    e = jnp.concatenate(
                        [pltpu.bitcast(pltpu.bitcast(e[:8], U32) | hold[:, :2 * L], F32), e[8:]], axis=0)
                pm[p] = e.astype(BF16)

            def attend(g):
                for p in range(2 * g - 4, 2 * g - 2) if g >= 2 else ():
                    o2 = _dot(pm[p], qkv(p, 2))
                    oc[p] = jnp.concatenate([o2[:SEG], o2[SEG:]], axis=1)
                for p in range(2 * g - 2, 2 * g) if 1 <= g <= NG else ():
                    score(p)

            def wo(p0, p1):
                rows = lambda p: jnp.concatenate([prev_rows[p], ov[p], oc[p]], axis=0) if sidx % 2 else oc[p]
                lhs = jnp.concatenate([rows(p) for p in range(p0, p1)], axis=1).astype(BF16)
                w = wo_ref[p0 * Dh:p1 * Dh, :]
                if any(k[0] == p0 for k in ogate):
                    top = [w[:8, n * 128:(n + 1) * 128] for n in range(D // 128)]
                    top = [c | ogate.pop((p0, n)) if (p0, n) in ogate else c for n, c in enumerate(top)]
                    w = jnp.concatenate([jnp.concatenate(top, axis=1), w[8:]], axis=0)
                t = _dot(lhs, _bf(w))
                acc[:] = [t + acc[0] if acc else t]

            fillers = [functools.partial(wo, *g) for g in wo_groups]
            fillers[3:3] = extra
            for g in range(NG):
                project(g)
            for g in range(NG, NG + 2):
                fillers.pop(0)()
                attend(g)
            for f in fillers:
                f()
            return acc[0], ov, early

        def step(it):
            r = _rows(it * TB, TB, TB)
            zero = jnp.maximum(it - NB, 0) * 8
            stage_ws(it, 0)
            us = [untranspose(_bf(u_ref[_rows(it * (FU // 2) + f0 // 2, HB, 8), 0:TB]).astype(F32))
                  for f0 in range(0, FU, TB)]
            NUP = len(us)
            done = lambda parts: functools.reduce(lambda a, b: a | b, [_token(_u32(u)[HB - 8:]) for u in parts])
            gate = []

            def rest(f0):
                us.append(untranspose(ut_part(it, 0, f0, min(f0 + TB, Fh))))

            def fin(n0, n1):
                y = _dot(jnp.concatenate(us[NUP:], axis=1), _bf(wout_ref[FU // 2:, n0:n1])) + y_up[:, n0:n1]
                gate.append(_silu(y))

            xs = _bf(xn_ref[_rows(it * HB, HB, HB), 0:D]).astype(F32)
            nx = _bf(xn_ref[_rows(jnp.minimum(it + 1, NB - 1) * HB, 8, 8), 0:D]).astype(F32)
            xs = jnp.concatenate([xs, nx[:M]], axis=0)

            def lhs(sidx, mem):
                x = xs[sidx * SEG:(sidx + 1) * SEG + M]
                return (jnp.concatenate([x[M:SEG], mem], axis=0).astype(BF16),
                        jnp.concatenate([x[:M], x[SEG:]], axis=0).astype(BF16))

            mem = lambda acc: acc[-M:].astype(BF16).astype(F32)
            even = ((0, 4), (4, 10), (10, 14), (14, 16))
            odd = ((0, 2), (2, 8), (8, 12), (12, 16))
            acc0, ov0, e0 = segment(0, *lhs(0, mem_ref[...]), lambda p: ear_ref[p // 2], None, [], even, zero,
                                    done(us))
            y_up = _dot(jnp.concatenate(us, axis=1), _bf(wout_ref[0:FU // 2, :]))
            acc1, _, e1 = segment(1, *lhs(1, mem(acc0)), e0.get, ov0,
                                  [lambda: rest(FU), lambda: rest(FU + TB)], odd, zero)
            rest(FU + 2 * TB)
            acc2, ov2, e2 = segment(2, *lhs(2, mem(acc1)), e1.get, None, [], even, zero, done(us[NUP:NUP + 2]))
            fin(0, 4 * 128)
            acc3, _, e3 = segment(3, *lhs(3, mem(acc2)), e2.get, ov2, [lambda: fin(4 * 128, D)], odd, zero)
            for p in e3:
                ear_ref[p // 2] = e3[p]
            mem_ref[...] = mem(acc3)
            sa = jnp.concatenate([acc1[:M], acc0[:SEG - M], acc1[M:SEG + M],
                                  acc3[:M], acc2[:SEG - M], acc3[M:SEG + M]], axis=0)
            o_ref[r, :] = (x_ref[r, :].astype(F32) + sa * jnp.concatenate(gate, axis=1)).astype(BF16)
            pltpu.make_async_copy(o_ref.at[r, :], o_hbm.at[r, :], osem).start()

        loop(NB, step)
        pltpu.make_async_copy(o_ref, o_hbm, osem).wait()

    any_spec = pl.BlockSpec(memory_space=pl.ANY)
    out = pl.pallas_call(
        kern,
        out_shape=jax.ShapeDtypeStruct((S, D), BF16),
        in_specs=[any_spec] * 10,
        out_specs=any_spec,
        scratch_shapes=[
            pltpu.VMEM((S, D), BF16),
            pltpu.VMEM((F // 2, D), U32),
            pltpu.VMEM((3 * H, D2, Dh), U32),
            pltpu.VMEM((H * Dh // 2, D), U32),
            pltpu.VMEM((HF, D), U32),
            pltpu.VMEM((S // 2, S), U32),
            pltpu.VMEM((S, D), BF16),
            pltpu.VMEM((S // 2, D + 128), U32),
            pltpu.VMEM((NB * HF, 2 * TB), U32),
            pltpu.VMEM((NB, 8, TB), F32),
            pltpu.VMEM((M, D), F32),
            pltpu.VMEM((NB * FU // 2, 2 * TB), U32),
            pltpu.VMEM((NB, Fh, TB), F32),
            pltpu.VMEM((FS * HB, D + 128), U32),
            pltpu.VMEM((GB, HB, S), U32),
            pltpu.VMEM((NP // 2, M, 6 * Dh), F32),
            pltpu.VMEM((M, D), BF16),
            pltpu.VMEM((NB, TB), BF16),
            pltpu.SemaphoreType.DMA((FI + 2,)),
            pltpu.SemaphoreType.DMA((NU,)),
            pltpu.SemaphoreType.DMA((NU,)),
            pltpu.SemaphoreType.DMA((7,)),
            pltpu.SemaphoreType.DMA,
        ] + [pltpu.VMEM((L, 3 * Dh), U32)] * NP,
        compiler_params=pltpu.CompilerParams(vmem_limit_bytes=120 * 1024 * 1024),
    )(x2, mem0, wq, wk, wv, wo, winT, B_w_sp, b2, B_w_out)
    return out.reshape(1, S, D)


def pallas_recurrent_scan__memory_aug_recurrent_mem_tr__mixer_gmlp__prompt_kernel(A_x, A_mem0, A_Wq, A_Wk, A_Wv, A_Wo, A_seg_len, B_x, B_w_in, B_w_sp, B_b_sp, B_w_out):
    del B_x
    seg = A_seg_len if isinstance(A_seg_len, int) else 32
    return _run(A_x, A_mem0, A_Wq, A_Wk, A_Wv, A_Wo, B_w_in, B_w_sp, B_b_sp, B_w_out, SEG=seg)
```
